```python
import jax
import jax.numpy as jnp

def _softmax(x, axis=-1):
    return jax.nn.softmax(x, axis=axis)
def _gelu(x):
    return jax.nn.gelu(x, approximate=True)
def _silu(x):
    return jax.nn.silu(x)
def _sigmoid(x):
    return jax.nn.sigmoid(x)
def _layernorm(x, axis=-1, eps=1e-5):
    m = jnp.mean(x, axis=axis, keepdims=True)
    v = jnp.var(x, axis=axis, keepdims=True)
    return (x - m) / jnp.sqrt(v + eps)
def _scatter_add(tgt, idx, src, axis=0):
    return tgt.at[idx].add(src)
def _segment_sum(src, seg, n):
    return jax.ops.segment_sum(src, seg, n)
class _Rng:
    def __init__(self, key):
        self._k = key
    def _next(self):
        self._k, sub = jax.random.split(self._k)
        return sub
    def normal(self, shape):
        return jax.random.normal(self._next(), shape, dtype=jnp.bfloat16)
    def randint(self, lo, hi, shape):
        return jax.random.randint(self._next(), shape, lo, hi, dtype=jnp.int32)
    def uniform(self, shape, lo=0.0, hi=1.0):
        return jax.random.uniform(self._next(), shape, jnp.bfloat16, lo, hi)
    def permutation(self, n):
        return jax.random.permutation(self._next(), n)


kernel_name = 'parallel_sum__sliding_local_dilated__mixer_token_mlp__prompt'

def setup_inputs():
    _rng = _Rng(jax.random.key(int.from_bytes(__import__("os").urandom(4), "little")))
    _w = (lambda a: (lambda t: t.astype(jnp.bfloat16) if jnp.issubdtype(t.dtype, jnp.floating) else t)(jnp.asarray(a)))
    def _A_setup():
        B, S, D = 1, 2048, 448
        return {
            "x": _w((lambda *s: _rng.normal(s) * 0.05)(B, S, D)),
            "wqkv": _w((lambda *s: _rng.normal(s) * 0.05)(D, 3 * D)),
            "wo": _w((lambda *s: _rng.normal(s) * 0.05)(D, D)),
        }
    _A_in = _A_setup()

    def _B_setup():
        B, S, D, F = 1, 2048, 448, 1792
        return {
            "x": _w((lambda *s: _rng.normal(s) * 0.05)(B, S, D)),
            "w1": _w((lambda *s: _rng.normal(s) * 0.05)(S, F) * (S ** -0.5)),
            "b1": _w((lambda *s: _rng.normal(s) * 0.05)(F) * 0.02),
            "w2": _w((lambda *s: _rng.normal(s) * 0.05)(F, S) * (F ** -0.5)),
            "b2": _w((lambda *s: _rng.normal(s) * 0.05)(S) * 0.02),
        }
    _B_in = _B_setup()

    return {
        "A_x": _A_in["x"],
        "A_wqkv": _A_in["wqkv"],
        "A_wo": _A_in["wo"],
        "B_x": _B_in["x"],
        "B_w1": _B_in["w1"],
        "B_b1": _B_in["b1"],
        "B_w2": _B_in["w2"],
        "B_b2": _B_in["b2"],
    }

def reference(A_x, A_wqkv, A_wo, B_x, B_w1, B_b1, B_w2, B_b2):
    def _A_ref(x, wqkv, wo):
        B, S, D = x.shape
        H = 16; Dh = D // H
        W, dil = 8, 2
        qkv = (lambda x, *d: x.transpose(*d))((x @ wqkv).reshape(B, S, 3, H, Dh), 2, 0, 3, 1, 4)
        q, k, v = qkv[0], qkv[1], qkv[2]
        scale = Dh ** -0.5
        pos = jnp.arange(S)
        off = jnp.arange(W) * dil
        idx = pos[:, None] - off[None, :]
        mask = idx >= 0
        idx_c = jnp.where(mask, idx, 0).reshape(-1)
        kg = k[:, :, idx_c, :].reshape(B, H, S, W, Dh)
        vg = v[:, :, idx_c, :].reshape(B, H, S, W, Dh)
        logits = jnp.einsum("bhsd,bhswd->bhsw", q, kg) * scale
        logits = jnp.where(mask[None, None, :, :], logits, -1e9)
        attn = _softmax(logits, axis=-1)
        o = jnp.einsum("bhsw,bhswd->bhsd", attn, vg)
        return (lambda x, *d: x.transpose(*d))(o, 0, 2, 1, 3).reshape(B, S, D) @ wo

    def _B_ref(x, w1, b1, w2, b2):
        B, S, D = x.shape
        h = _layernorm(x, axis=-1)
        u = jnp.einsum("bsd,sf->bdf", h, w1) + b1
        u = _gelu(u)
        y = jnp.einsum("bdf,fs->bds", u, w2) + b2
        return (lambda x, *d: x.transpose(*d))(y, 0, 2, 1)

    x = A_x
    xn = _layernorm(x, axis=-1)
    return x + _A_ref(xn, A_wqkv, A_wo) + _B_ref(xn, B_w1, B_b1, B_w2, B_b2)
```

```python
import jax
import jax.numpy as jnp
import numpy as np
import jax.experimental.pallas as pl
import jax.experimental.pallas.tpu as pltpu

S, D, H, DH, F = 2048, 448, 16, 28, 1792
W, DIL = 8, 2
NT = S // 128
EPS = 1e-5
f32, bf16, u32 = jnp.float32, jnp.bfloat16, jnp.uint32


def _unpack(x, i):
    return pltpu.unpack_elementwise(x, index=i, packed_dtype=bf16, unpacked_dtype=f32)


def _pack(a, b):
    return pltpu.pack_elementwise([a, b], packed_dtype=bf16)


def _tree_sum(xs):
    xs = list(xs)
    while len(xs) > 1:
        nxt = [xs[i] + xs[i + 1] for i in range(0, len(xs) - 1, 2)]
        if len(xs) % 2:
            nxt.append(xs[-1])
        xs = nxt
    return xs[0]


def _bcast_rows_sum(p):
    t = jnp.sum(p, axis=0, keepdims=True)
    return jnp.broadcast_to(t, (8, 128))


def _ln_stats(vals):
    mean = _bcast_rows_sum(_tree_sum(vals)) * (1.0 / D)
    c = [v - mean for v in vals]
    var = _bcast_rows_sum(_tree_sum([t * t for t in c])) * (1.0 / D)
    return c, jax.lax.rsqrt(var + EPS)


def _kernel(x_hbm, wqkv_hbm, wo_hbm, w1_hbm, b1_hbm, w2_hbm, b2_hbm, out_hbm,
            x_s, wqkv_s, wo_s, w1_s, w2_s, b1_s, b2_s,
            wt_f, wo_f, wt_s, wot_s,
            xn_s, h_s, q_s, k_s, v_s, o_s, r_s, u_s, ub_s, out_s, sems):
    sem_i = [0]

    def dma(src, dst):
        c = pltpu.make_async_copy(src, dst, sems.at[sem_i[0]])
        sem_i[0] += 1
        c.start()
        return c

    KB = 4
    NB = NT // KB
    cp_x = [None] * NT
    cp_w1 = [None] * NB
    for j in range(KB):
        cp_x[j] = dma(x_hbm.at[:, pl.ds(128 * j, 128)], x_s.at[j])
    cp_wqkv = dma(wqkv_hbm, wqkv_s)
    cp_w1[0] = dma(w1_hbm.at[pl.ds(0, 128 * KB)], w1_s.at[pl.ds(0, 128 * KB)])
    cp_wo = dma(wo_hbm, wo_s)
    cp_b1 = dma(b1_hbm, b1_s)
    cp_b2 = dma(b2_hbm, b2_s)
    for b in range(1, NB):
        for j in range(KB * b, KB * b + KB):
            cp_x[j] = dma(x_hbm.at[:, pl.ds(128 * j, 128)], x_s.at[j])
        cp_w1[b] = dma(w1_hbm.at[pl.ds(128 * KB * b, 128 * KB)], w1_s.at[pl.ds(128 * KB * b, 128 * KB)])
    W2B = 4
    cp_w2 = [dma(w2_hbm.at[:, pl.ds(512 * b, 512)], w2_s.at[:, pl.ds(512 * b, 512)]) for b in range(S // 512)]

    lane = jax.lax.broadcasted_iota(jnp.int32, (8, 128), 1)

    def layer_norms(j):
        xp = [pltpu.bitcast(x_s[j, 16 * i:16 * i + 16, :], u32) for i in range(D // 16)]
        vals = [_unpack(p, t) for p in xp for t in range(2)]
        c, rstd = _ln_stats(vals)
        xn = [t * rstd for t in c]
        xnp = [_pack(xn[2 * i], xn[2 * i + 1]) for i in range(D // 16)]
        for i in range(D // 16):
            xn_s[j, 16 * i:16 * i + 16, :] = pltpu.bitcast(xnp[i], bf16)
        vals2 = [_unpack(p, t) for p in xnp for t in range(2)]
        c2, rstd2 = _ln_stats(vals2)
        for i in range(D // 16):
            hp = _pack(c2[2 * i] * rstd2, c2[2 * i + 1] * rstd2)
            h_s[j, 16 * i:16 * i + 16, :] = pltpu.bitcast(hp, bf16)

    def prep_wqkv():
        for c in range(4):
            rows = min(128, D - 128 * c)
            w = wqkv_s[128 * c:128 * c + rows, :].astype(f32)
            if rows < 128:
                w = jnp.concatenate([w, jnp.zeros((128 - rows, 3 * D), f32)], axis=0)
            wt_f[c] = w.T
        for c in range(4):
            for sec in range(3):
                for d in range(DH):
                    parts = [wt_f[c, pl.ds(sec * D + DH * g + d, 8, stride=2 * DH), :] for g in range(2)]
                    wt_s[c, sec * D + 16 * d:sec * D + 16 * d + 16, :] = jnp.concatenate(parts, axis=0).astype(bf16)

    def prep_wo():
        for c in range(4):
            cols = min(128, D - 128 * c)
            w = wo_s[:, 128 * c:128 * c + cols].astype(f32)
            if cols < 128:
                w = jnp.concatenate([w, jnp.zeros((D, 128 - cols), f32)], axis=1)
            wo_f[c] = w
        for c in range(4):
            parts = []
            for d in range(DH):
                for m in range(2):
                    parts.append(wo_f[c, pl.ds(DH * 8 * m + d, 8, stride=DH), :])
            wp = jnp.concatenate(parts, axis=0)
            wp = jnp.concatenate([wp, jnp.zeros((512 - D, 128), f32)], axis=0)
            wpt = wp.T
            rows = min(128, D - 128 * c)
            for cc in range(4):
                wot_s[cc, 128 * c:128 * c + rows, :] = wpt[:rows, 128 * cc:128 * cc + 128].astype(bf16)

    def lhs_448(ref, rows):
        return jnp.concatenate([ref[0], ref[1], ref[2], ref[3, :, 0:64]], axis=1)

    def qkv(j):
        wt = lhs_448(wt_s, 3 * D)
        res = jnp.dot(wt, xn_s[j], preferred_element_type=f32)
        q_s[j] = res[0:D]
        for d in range(DH):
            k_s[j, 8 * d:8 * d + 8, :] = _pack(res[D + 16 * d:D + 16 * d + 8], res[D + 16 * d + 8:D + 16 * d + 16])
            v_s[j, 8 * d:8 * d + 8, :] = _pack(res[2 * D + 16 * d:2 * D + 16 * d + 8], res[2 * D + 16 * d + 8:2 * D + 16 * d + 16])

    def shifted(cur, prev, w):
        if w == 0:
            return cur
        sh = DIL * w
        return pltpu.roll(jnp.where(lane >= 128 - sh, prev, cur), sh, 1)

    def attention(j):
        jp = max(j - 1, 0)
        acc = [[None, None] for _ in range(W)]
        for d in range(DH):
            q = [q_s[j, 16 * d + 8 * g:16 * d + 8 * g + 8, :] for g in range(2)]
            k = k_s[j, 8 * d:8 * d + 8, :]
            kp = k_s[jp, 8 * d:8 * d + 8, :]
            for w in range(W):
                ks = shifted(k, kp, w)
                for g in range(2):
                    p = q[g] * _unpack(ks, g)
                    acc[w][g] = p if acc[w][g] is None else acc[w][g] + p
        scale = DH ** -0.5
        prob = [[None, None] for _ in range(W)]
        for g in range(2):
            lg = [acc[w][g] * scale for w in range(W)]
            if j == 0:
                lg = [lg[w] if w == 0 else jnp.where(lane >= DIL * w, lg[w], -1e9) for w in range(W)]
            m = lg[0]
            for w in range(1, W):
                m = jnp.maximum(m, lg[w])
            e = [jnp.exp(t - m) for t in lg]
            inv = 1.0 / _tree_sum(e)
            for w in range(W):
                prob[w][g] = e[w] * inv
        for d in range(DH):
            v = v_s[j, 8 * d:8 * d + 8, :]
            vp = v_s[jp, 8 * d:8 * d + 8, :]
            o = [None, None]
            for w in range(W):
                vs = shifted(v, vp, w)
                for g in range(2):
                    p = prob[w][g] * _unpack(vs, g)
                    o[g] = p if o[g] is None else o[g] + p
            o_s[j, 16 * d:16 * d + 16, :] = pltpu.bitcast(_pack(o[0], o[1]), bf16)

    def oproj(j):
        wot = lhs_448(wot_s, D)
        a = jnp.dot(wot, o_s[j], preferred_element_type=f32)
        b2 = b2_s[pl.ds(128 * j, 128)].astype(f32).reshape(1, 128)
        r_s[j] = a + x_s[j].astype(f32) + b2

    def mixer_up(b):
        hb = jnp.concatenate([h_s[j] for j in range(KB * b, KB * b + KB)], axis=1)
        upd = jnp.dot(hb, w1_s[128 * KB * b:128 * KB * (b + 1), :], preferred_element_type=f32)
        if b == 0:
            u_s[...] = upd
        else:
            u_s[...] = u_s[...] + upd

    def gelu_all():
        b1 = b1_s[...].astype(f32).reshape(1, F)
        for c in range(F // 128):
            t = u_s[:, 128 * c:128 * c + 128] + b1[:, 128 * c:128 * c + 128]
            ub_s[c] = jax.nn.gelu(t, approximate=True).astype(bf16)

    def mixer_down(j0, nj):
        ub = jnp.concatenate([ub_s[c] for c in range(F // 128)], axis=1)
        y = jnp.dot(ub, w2_s[:, 128 * j0:128 * (j0 + nj)], preferred_element_type=f32)
        for t in range(nj):
            out_s[j0 + t] = (y[:, 128 * t:128 * t + 128] + r_s[j0 + t]).astype(bf16)

    for j in range(KB):
        cp_x[j].wait()
        layer_norms(j)
    cp_wqkv.wait()
    prep_wqkv()
    cp_w1[0].wait()
    cp_wo.wait()
    cp_b1.wait()
    cp_b2.wait()
    prep_wo()
    for b in range(NB):
        if b > 0:
            for j in range(KB * b, KB * b + KB):
                cp_x[j].wait()
            cp_w1[b].wait()
            for j in range(KB * b, KB * b + KB):
                layer_norms(j)
        mixer_up(b)
        for j in range(KB * b, KB * b + KB):
            qkv(j)
            attention(j)
            oproj(j)
    gelu_all()
    for c in cp_w2:
        c.wait()
    cp_out = []
    for j0 in range(0, NT, 2):
        mixer_down(j0, 2)
        for j in (j0, j0 + 1):
            cp_out.append(dma(out_s.at[j], out_hbm.at[:, pl.ds(128 * j, 128)]))
    for c in cp_out:
        c.wait()


N_SEMS = NT + 4 + 4 + 4 + NT


@jax.jit
def pallas_parallel_sum__sliding_local_dilated__mixer_token_mlp__prompt_kernel(
    A_x, A_wqkv, A_wo, B_x, B_w1, B_b1, B_w2, B_b2,
):
    del B_x
    xT = A_x.reshape(S, D).T
    any_spec = pl.BlockSpec(memory_space=pl.ANY)
    scratch = [
        pltpu.VMEM((NT, D, 128), bf16),
        pltpu.VMEM((D, 3 * D), bf16),
        pltpu.VMEM((D, D), bf16),
        pltpu.VMEM((S, F), bf16),
        pltpu.VMEM((F, S), bf16),
        pltpu.VMEM((F,), bf16),
        pltpu.VMEM((S,), bf16),
        pltpu.VMEM((4, 3 * D, 128), f32),
        pltpu.VMEM((4, D, 128), f32),
        pltpu.VMEM((4, 3 * D, 128), bf16),
        pltpu.VMEM((4, D, 128), bf16),
        pltpu.VMEM((NT, D, 128), bf16),
        pltpu.VMEM((NT, D, 128), bf16),
        pltpu.VMEM((NT, D, 128), f32),
        pltpu.VMEM((NT, D // 2, 128), u32),
        pltpu.VMEM((NT, D // 2, 128), u32),
        pltpu.VMEM((NT, D, 128), bf16),
        pltpu.VMEM((NT, D, 128), f32),
        pltpu.VMEM((D, F), f32),
        pltpu.VMEM((F // 128, D, 128), bf16),
        pltpu.VMEM((NT, D, 128), bf16),
        pltpu.SemaphoreType.DMA((N_SEMS,)),
    ]
    outT = pl.pallas_call(
        _kernel,
        out_shape=jax.ShapeDtypeStruct((D, S), bf16),
        in_specs=[any_spec] * 7,
        out_specs=any_spec,
        scratch_shapes=scratch,
        compiler_params=pltpu.CompilerParams(vmem_limit_bytes=100 * 1024 * 1024),
        name="fused_kernel",
    )(xT, A_wqkv, A_wo, B_w1, B_b1, B_w2, B_b2)
    return outT.T.reshape(1, S, D)
```

```python
import jax
import jax.numpy as jnp
import numpy as np
import jax.experimental.pallas as pl
import jax.experimental.pallas.tpu as pltpu

S, D, H, DH, F = 2048, 448, 16, 28, 1792
W, DIL = 8, 2
NT = S // 128
NF = F // 128
EPS = 1e-5
f32, bf16, u32, i32 = jnp.float32, jnp.bfloat16, jnp.uint32, jnp.int32


def _unpack(x, i):
    return pltpu.unpack_elementwise(x, index=i, packed_dtype=bf16, unpacked_dtype=f32)


def _unpack2(x, i):
    if i == 0:
        return jax.lax.bitcast_convert_type(x << 16, f32)
    return jax.lax.bitcast_convert_type(x & jnp.uint32(0xFFFF0000), f32)


def _pack(a, b):
    return pltpu.pack_elementwise([a, b], packed_dtype=bf16)


def _as_bf16(x_u32):
    return pltpu.bitcast(x_u32, bf16)


def _tree_sum(xs):
    xs = list(xs)
    while len(xs) > 1:
        nxt = [xs[i] + xs[i + 1] for i in range(0, len(xs) - 1, 2)]
        if len(xs) % 2:
            nxt.append(xs[-1])
        xs = nxt
    return xs[0]


def _bcast_rows_sum(p):
    t = jnp.sum(p, axis=0, keepdims=True)
    return jnp.broadcast_to(t, (8, 128))


def _never(tok):
    return tok * tok < -1.0


def _zero_after(tok):
    return jnp.where(_never(tok), 1.0, 0.0).astype(f32)


KB = 4
NB = NT // KB
LOOP_N, LOOP_P = (2, 3)
LN_AT = (6, 8, 10, 12)
PREP_WO_AT = (4, 5, 7, 9)
PREP_AT = (4, 8, 12, 13)
FLAGS = {"XLA_TPU_RESCHEDULE_DMA_DONES": True}
N_SEMS = 64


def _kernel(x_hbm, wqkv_hbm, wo_hbm, w1_hbm, b1_hbm, w2_hbm, b2_hbm, out_hbm,
            x_s, wqkv_s, wo_s, w1_s, w2_s, b1_s, b2_s,
            wt_f, wo_f, wt_s, wot_s,
            xn_s, h_s, q_s, k_s, v_s, o_s, r_s, u_s, ub_s, out_s, sems):
    x_hbm, wqkv_hbm, wo_hbm, w1_hbm, w2_hbm, out_hbm = (
        r.bitcast(u32) for r in (x_hbm, wqkv_hbm, wo_hbm, w1_hbm, w2_hbm, out_hbm))
    sem_i = [0]

    class Dma:
        def __init__(self, src, dst):
            self.src, self.dst, self.i = src, dst, sem_i[0]
            sem_i[0] += 1
            pltpu.make_async_copy(src, dst, sems.at[self.i]).start()

        def wait(self, tok=None):
            idx = self.i
            if tok is not None:
                idx = idx + jnp.where(_never(tok), 1, 0).astype(i32)[0, 0]
            pltpu.make_async_copy(self.src, self.dst, sems.at[idx]).wait()

    def lt(j, n=1):
        return slice(128 * j, 128 * (j + n))

    def x_dma(j, n):
        return Dma(x_hbm.at[:, lt(j, n)], x_s.at[:, lt(j, n)])

    def w1_dma(b, c0=0, n=NF):
        rows = pl.ds(64 * KB * b, 64 * KB)
        return Dma(w1_hbm.at[rows, lt(c0, n)], w1_s.at[rows, lt(c0, n)])

    def wqkv_dma(c):
        rows = pl.ds(64 * c, min(64, D // 2 - 64 * c))
        return Dma(wqkv_hbm.at[rows], wqkv_s.at[rows])

    cp_xt = [x_dma(j, 1) for j in range(KB)]
    cp_w10, cp_wqkv = [], []
    for i in range(NF // 2):
        cp_w10.append(w1_dma(0, 2 * i, 2))
        if i in (2, 4):
            cp_wqkv.append(wqkv_dma(len(cp_wqkv)))
    cp_wqkv += [wqkv_dma(2), wqkv_dma(3)]
    cp_x1 = x_dma(KB, KB)
    cp_w1 = [None, w1_dma(1)]
    cp_wo = Dma(wo_hbm, wo_s)
    cp_b2 = Dma(b2_hbm, b2_s)
    cp_x2 = x_dma(2 * KB, KB)
    cp_x3 = x_dma(3 * KB, KB)
    cp_b1 = Dma(b1_hbm, b1_s)
    cp_w1 += [w1_dma(2), w1_dma(3)]
    cp_w2 = [Dma(w2_hbm.at[:, lt(4 * b, 4)], w2_s.at[:, lt(4 * b, 4)]) for b in range(4)]

    lane = jax.lax.broadcasted_iota(jnp.int32, (8, 128), 1)

    def layer_norms(j, dep=None):
        n16 = D // 16
        k0 = jnp.broadcast_to(_unpack(x_s[0:8, lt(j)], 0)[0:1, :], (8, 128))
        if dep is not None:
            k0 = k0 + _zero_after(dep)
        s1, s2 = [None, None], [None, None]
        for i in range(n16):
            p = x_s[8 * i:8 * i + 8, lt(j)]
            for t in range(2):
                c = _unpack(p, t) - k0
                s1[t] = c if s1[t] is None else s1[t] + c
                s2[t] = c * c if s2[t] is None else s2[t] + c * c
        m1 = _bcast_rows_sum(s1[0] + s1[1]) * (1.0 / D)
        m2 = _bcast_rows_sum(s2[0] + s2[1]) * (1.0 / D)
        mean = k0 + m1
        rstd = jax.lax.rsqrt(jnp.maximum(m2 - m1 * m1, 0.0) + EPS)
        t1, t2 = [None, None], [None, None]
        for i in range(n16):
            p = x_s[8 * i:8 * i + 8, lt(j)]
            xs = []
            for t in range(2):
                xn = (_unpack2(p, t) - mean) * rstd
                xs.append(xn)
                t1[t] = xn if t1[t] is None else t1[t] + xn
                t2[t] = xn * xn if t2[t] is None else t2[t] + xn * xn
            xn_s[8 * i:8 * i + 8, lt(j)] = _pack(xs[0], xs[1])
        mean2 = _bcast_rows_sum(t1[0] + t1[1]) * (1.0 / D)
        e2 = _bcast_rows_sum(t2[0] + t2[1]) * (1.0 / D)
        rstd2 = jax.lax.rsqrt(jnp.maximum(e2 - mean2 * mean2, 0.0) + EPS)
        for i in range(n16):
            p = xn_s[8 * i:8 * i + 8, lt(j)]
            h_s[8 * i:8 * i + 8, lt(j)] = _pack((_unpack(p, 0) - mean2) * rstd2, (_unpack(p, 1) - mean2) * rstd2)
        return rstd2

    def store_rows_bf16(ref, c, row0, val):
        ref[c, row0 // 2:(row0 + val.shape[0]) // 2, :] = pltpu.bitcast(val.astype(bf16), u32)

    def prep_wqkv(c, dep):
        rows = min(128, D - 128 * c)
        w = _as_bf16(wqkv_s[64 * c:64 * c + rows // 2, :]).astype(f32)
        w = w + jnp.tile(_zero_after(dep), (rows // 8, 11))[:, :3 * D]
        if rows < 128:
            w = jnp.concatenate([w, jnp.zeros((128 - rows, 3 * D), f32)], axis=0)
        wt_f[c] = w.T
        for sec in range(3):
            for d in range(DH):
                parts = [wt_f[c, pl.ds(sec * D + DH * g + d, 8, stride=2 * DH), :] for g in range(2)]
                store_rows_bf16(wt_s, c, sec * D + 16 * d, jnp.concatenate(parts, axis=0))

    def prep_wo(c, dep):
        cols = min(128, D - 128 * c)
        w = _as_bf16(wo_s[:, 128 * c:128 * c + cols]).astype(f32)
        w = w + jnp.tile(_zero_after(dep), (D // 8, 1))[:, :cols]
        if cols < 128:
            w = jnp.concatenate([w, jnp.zeros((D, 128 - cols), f32)], axis=1)
        wo_f[c] = w
        parts = []
        for d in range(DH):
            for m in range(2):
                parts.append(wo_f[c, pl.ds(DH * 8 * m + d, 8, stride=DH), :])
        wp = jnp.concatenate(parts, axis=0)
        wp = jnp.concatenate([wp, jnp.zeros((512 - D, 128), f32)], axis=0)
        wpt = wp.T
        rows = min(128, D - 128 * c)
        for cc in range(4):
            store_rows_bf16(wot_s, cc, 128 * c, wpt[:rows, lt(cc)])

    def lhs_448(ref, r0, nr):
        rs = slice(r0 // 2, (r0 + nr) // 2)
        return jnp.concatenate([_as_bf16(ref[0, rs, :]), _as_bf16(ref[1, rs, :]), _as_bf16(ref[2, rs, :]),
                                _as_bf16(ref[3, rs, :])[:, 0:64]], axis=1)

    def qkv(j, sec):
        wt = lhs_448(wt_s, sec * D, D)
        res = jnp.dot(wt, _as_bf16(xn_s[:, lt(j)]), preferred_element_type=f32)
        if sec == 0:
            q_s[j] = res
        else:
            dst = k_s if sec == 1 else v_s
            for d in range(DH):
                dst[j, 8 * d:8 * d + 8, :] = _pack(res[16 * d:16 * d + 8], res[16 * d + 8:16 * d + 16])
        return res[0:8]

    def shifted(cur, prev, w):
        if w == 0:
            return cur
        sh = DIL * w
        return pltpu.roll(jnp.where(lane >= 128 - sh, prev, cur), sh, 1)

    def attention(j):
        jp = max(j - 1, 0)
        acc = [[None, None] for _ in range(W)]
        for d in range(DH):
            q = [q_s[j, 16 * d + 8 * g:16 * d + 8 * g + 8, :] for g in range(2)]
            k = k_s[j, 8 * d:8 * d + 8, :]
            kp = k_s[jp, 8 * d:8 * d + 8, :]
            for w in range(W):
                ks = shifted(k, kp, w)
                for g in range(2):
                    p = q[g] * _unpack(ks, g)
                    acc[w][g] = p if acc[w][g] is None else acc[w][g] + p
        scale = DH ** -0.5
        prob = [[None, None] for _ in range(W)]
        for g in range(2):
            lg = [acc[w][g] * scale for w in range(W)]
            if j == 0:
                lg = [lg[w] if w == 0 else jnp.where(lane >= DIL * w, lg[w], -1e9) for w in range(W)]
            m = lg[0]
            for w in range(1, W):
                m = jnp.maximum(m, lg[w])
            e = [jnp.exp(t - m) for t in lg]
            inv = 1.0 / _tree_sum(e)
            for w in range(W):
                prob[w][g] = e[w] * inv
        for d in range(DH):
            v = v_s[j, 8 * d:8 * d + 8, :]
            vp = v_s[jp, 8 * d:8 * d + 8, :]
            o = [None, None]
            for w in range(W):
                vs = shifted(v, vp, w)
                for g in range(2):
                    p = prob[w][g] * _unpack(vs, g)
                    o[g] = p if o[g] is None else o[g] + p
            o_s[j, 8 * d:8 * d + 8, :] = _pack(o[0], o[1])

    def oproj(j):
        wot = lhs_448(wot_s, 0, D)
        a = jnp.dot(wot, _as_bf16(o_s[j]), preferred_element_type=f32)
        b2 = b2_s[pl.ds(128 * j, 128)].astype(f32).reshape(1, 128)
        r_s[j] = a + _as_bf16(x_s[:, lt(j)]).astype(f32) + b2

    def mixer_up(b, c):
        hb = _as_bf16(h_s[:, lt(KB * b, KB)])
        wb = _as_bf16(w1_s[64 * KB * b:64 * KB * (b + 1), lt(c)])
        upd = jnp.dot(hb, wb, preferred_element_type=f32)
        if b == 0:
            u_s[:, lt(c)] = upd
        elif b < NB - 1:
            u_s[:, lt(c)] = u_s[:, lt(c)] + upd
        else:
            b1 = b1_s[pl.ds(128 * c, 128)].astype(f32).reshape(1, 128)
            t = u_s[:, lt(c)] + upd + b1
            ub_s[:, lt(c)] = pltpu.bitcast(jax.nn.gelu(t, approximate=True).astype(bf16), u32)
        return upd[0:8]

    def mixer_down(j0, nj):
        ub = _as_bf16(ub_s[...])
        if isinstance(j0, int):
            cols = lambda t, n: lt(j0 + t, n)
        else:
            cols = lambda t, n: pl.ds(pl.multiple_of((j0 + t) * 128, 128), 128 * n)
        y = jnp.dot(ub, _as_bf16(w2_s[:, cols(0, nj)]), preferred_element_type=f32)
        for t in range(nj):
            out_s[:, cols(t, 1)] = pltpu.bitcast((y[:, lt(t)] + r_s[j0 + t]).astype(bf16), u32)

    def tiles(b):
        return range(KB * b, KB * b + KB)

    tok = None
    for j in tiles(0):
        cp_xt[j].wait(tok)
        tok = layer_norms(j)
    for c in range(NF):
        if c % 2 == 0:
            cp_w10[c // 2].wait(tok)
        tok = mixer_up(0, c)
        if c in PREP_AT:
            i = PREP_AT.index(c)
            cp_wqkv[i].wait(tok)
            prep_wqkv(i, tok)

    def out_copy(j0, n, sem):
        if isinstance(j0, int):
            sl = lt(j0, n)
        else:
            sl = pl.ds(pl.multiple_of(j0 * 128, 128), 128 * n)
        return pltpu.make_async_copy(out_s.at[:, sl], out_hbm.at[:, sl], sems.at[sem])

    for b in range(NB):
        for t, j in enumerate(tiles(b)):
            for sec in range(3):
                tok = qkv(j, sec)
                if b == 0 and t == 0 and sec == 0:
                    cp_x1.wait(tok)
                if b == 0 and sec == 1:
                    layer_norms(KB + t, tok)
                if t == KB - 1 and sec == 1:
                    if b + 1 < NB:
                        cp_w1[b + 1].wait(tok)
                    else:
                        for c in cp_w2:
                            c.wait(tok)
            attention(j)
        if b + 1 < NB:
            ln_at = dict(zip(LN_AT, tiles(b + 2))) if b + 2 < NB else {}
            for c in range(NF):
                tok = mixer_up(b + 1, c)
                if b == 0:
                    if c == 2:
                        cp_wo.wait(tok)
                        cp_b2.wait(tok)
                    if c == 4:
                        cp_x2.wait(tok)
                    if c in PREP_WO_AT:
                        prep_wo(PREP_WO_AT.index(c), tok)
                if b == 1 and c == 2:
                    cp_x3.wait(tok)
                    cp_b1.wait(tok)
                if c in ln_at:
                    layer_norms(ln_at[c], tok)
            for j in tiles(b):
                oproj(j)
        else:
            mixer_down(0, 2)
            for j in tiles(b):
                oproj(j)
    s0 = sem_i[0]
    out_copy(0, 2, s0).start()

    def body(i, carry):
        j0 = 2 + 2 * LOOP_P * i
        for p in range(LOOP_P):
            mixer_down(j0 + 2 * p, 2)
        out_copy(j0, 2 * LOOP_P, s0 + 1 + i).start()
        return carry

    jax.lax.fori_loop(0, LOOP_N, body, 0)
    jt = 2 + 2 * LOOP_P * LOOP_N
    for j0 in range(jt, NT, 2):
        mixer_down(j0, 2)
    out_copy(jt, NT - jt, s0 + 1 + LOOP_N).start()
    out_copy(0, 2, s0).wait()
    for i in range(LOOP_N):
        out_copy(2 + 2 * LOOP_P * i, 2 * LOOP_P, s0 + 1 + i).wait()
    out_copy(jt, NT - jt, s0 + 1 + LOOP_N).wait()


@jax.jit
def pallas_parallel_sum__sliding_local_dilated__mixer_token_mlp__prompt_kernel(
    A_x, A_wqkv, A_wo, B_x, B_w1, B_b1, B_w2, B_b2,
):
    del B_x
    xT = A_x.reshape(S, D).T
    any_spec = pl.BlockSpec(memory_space=pl.ANY)
    scratch = [
        pltpu.VMEM((D // 2, S), u32),
        pltpu.VMEM((D // 2, 3 * D), u32),
        pltpu.VMEM((D // 2, D), u32),
        pltpu.VMEM((S // 2, F), u32),
        pltpu.VMEM((F // 2, S), u32),
        pltpu.VMEM((F,), bf16),
        pltpu.VMEM((S,), bf16),
        pltpu.VMEM((4, 3 * D, 128), f32),
        pltpu.VMEM((4, D, 128), f32),
        pltpu.VMEM((4, 3 * D // 2, 128), u32),
        pltpu.VMEM((4, D // 2, 128), u32),
        pltpu.VMEM((D // 2, S), u32),
        pltpu.VMEM((D // 2, S), u32),
        pltpu.VMEM((NT, D, 128), f32),
        pltpu.VMEM((NT, D // 2, 128), u32),
        pltpu.VMEM((NT, D // 2, 128), u32),
        pltpu.VMEM((NT, D, 128), u32),
        pltpu.VMEM((NT, D, 128), f32),
        pltpu.VMEM((D, F), f32),
        pltpu.VMEM((D // 2, F), u32),
        pltpu.VMEM((D // 2, S), u32),
        pltpu.SemaphoreType.DMA((N_SEMS,)),
    ]
    scratch[16] = pltpu.VMEM((NT, D // 2, 128), u32)
    outT = pl.pallas_call(
        _kernel,
        out_shape=jax.ShapeDtypeStruct((D, S), bf16),
        in_specs=[any_spec] * 7,
        out_specs=any_spec,
        scratch_shapes=scratch,
        compiler_params=pltpu.CompilerParams(vmem_limit_bytes=100 * 1024 * 1024, flags=FLAGS),
        name="fused_kernel",
    )(xT, A_wqkv, A_wo, B_w1, B_b1, B_w2, B_b2)
    return outT.T.reshape(1, S, D)
```

```python
import jax
import jax.numpy as jnp
import numpy as np
import jax.experimental.pallas as pl
import jax.experimental.pallas.tpu as pltpu

S, D, H, DH, F = 2048, 448, 16, 28, 1792
W, DIL = 8, 2
NT = S // 128
NF = F // 128
EPS = 1e-5
f32, bf16, u32, i32 = jnp.float32, jnp.bfloat16, jnp.uint32, jnp.int32


def _unpack(x, i):
    return pltpu.unpack_elementwise(x, index=i, packed_dtype=bf16, unpacked_dtype=f32)


def _unpack2(x, i):
    if i == 0:
        return jax.lax.bitcast_convert_type(x << 16, f32)
    return jax.lax.bitcast_convert_type(x & jnp.uint32(0xFFFF0000), f32)


def _pack(a, b):
    return pltpu.pack_elementwise([a, b], packed_dtype=bf16)


def _as_bf16(x_u32):
    return pltpu.bitcast(x_u32, bf16)


def _tree_sum(xs):
    xs = list(xs)
    while len(xs) > 1:
        nxt = [xs[i] + xs[i + 1] for i in range(0, len(xs) - 1, 2)]
        if len(xs) % 2:
            nxt.append(xs[-1])
        xs = nxt
    return xs[0]


def _bcast_rows_sum(p):
    t = jnp.sum(p, axis=0, keepdims=True)
    return jnp.broadcast_to(t, (8, 128))


def _never(tok):
    return tok * tok < -1.0


def _zero_after(tok):
    return jnp.where(_never(tok), 1.0, 0.0).astype(f32)


KB = 4
NB = NT // KB
LOOP_N, LOOP_P = (2, 3)
LN_AT = (6, 8, 10, 12)
PREP_WO_AT = (4, 5, 7, 9)
PREP_AT = (4, 8, 12, 12)
LNQ_AT = (1, 2, 3, 4)
FLAGS = {"XLA_TPU_RESCHEDULE_DMA_DONES": True, "XLA_TPU_EVENLY_DISTRIBUTE_CRITICAL_NODES": True}
N_SEMS = 64


def _kernel(x_hbm, wqkv_hbm, wo_hbm, w1_hbm, b1_hbm, w2_hbm, b2_hbm, out_hbm,
            x_s, wqkv_s, wo_s, w1_s, w2_s, b1_s, b2_s,
            wt_f, wo_f, wt_s, wot_s,
            xn_s, h_s, q_s, k_s, v_s, o_s, r_s, u_s, ub_s, out_s, sems):
    x_hbm, wqkv_hbm, wo_hbm, w1_hbm, w2_hbm, out_hbm = (
        r.bitcast(u32) for r in (x_hbm, wqkv_hbm, wo_hbm, w1_hbm, w2_hbm, out_hbm))
    sem_i = [0]

    class Dma:
        def __init__(self, src, dst):
            self.src, self.dst, self.i = src, dst, sem_i[0]
            sem_i[0] += 1
            pltpu.make_async_copy(src, dst, sems.at[self.i]).start()

        def wait(self, tok=None):
            idx = self.i
            if tok is not None:
                idx = idx + jnp.where(_never(tok), 1, 0).astype(i32)[0, 0]
            pltpu.make_async_copy(self.src, self.dst, sems.at[idx]).wait()

    def lt(j, n=1):
        return slice(128 * j, 128 * (j + n))

    def x_dma(j, n):
        return Dma(x_hbm.at[:, lt(j, n)], x_s.at[:, lt(j, n)])

    def w1_dma(b, c0=0, n=NF):
        rows = pl.ds(64 * KB * b, 64 * KB)
        return Dma(w1_hbm.at[rows, lt(c0, n)], w1_s.at[rows, lt(c0, n)])

    def wqkv_dma(c):
        rows = pl.ds(64 * c, min(64, D // 2 - 64 * c))
        return Dma(wqkv_hbm.at[rows], wqkv_s.at[rows])

    cp_xt = [x_dma(j, 1) for j in range(KB)]
    cp_w10, cp_wqkv = [], []
    for i in range(NF // 2):
        cp_w10.append(w1_dma(0, 2 * i, 2))
        if i in (2, 4):
            cp_wqkv.append(wqkv_dma(len(cp_wqkv)))
    cp_wqkv += [wqkv_dma(2), wqkv_dma(3)]
    cp_x1 = x_dma(KB, KB)
    cp_w1 = [None, w1_dma(1)]
    cp_wo = Dma(wo_hbm, wo_s)
    cp_b2 = Dma(b2_hbm, b2_s)
    cp_x2 = x_dma(2 * KB, KB)
    cp_x3 = x_dma(3 * KB, KB)
    cp_b1 = Dma(b1_hbm, b1_s)
    cp_w1 += [w1_dma(2), w1_dma(3)]
    cp_w2 = [Dma(w2_hbm.at[:, lt(4 * b, 4)], w2_s.at[:, lt(4 * b, 4)]) for b in range(4)]

    lane = jax.lax.broadcasted_iota(jnp.int32, (8, 128), 1)

    def layer_norms(j, dep=None):
        n16 = D // 16
        k0 = jnp.broadcast_to(_unpack(x_s[0:8, lt(j)], 0)[0:1, :], (8, 128))
        if dep is not None:
            k0 = k0 + _zero_after(dep)
        s1, s2 = [None, None], [None, None]
        for i in range(n16):
            p = x_s[8 * i:8 * i + 8, lt(j)]
            for t in range(2):
                c = _unpack(p, t) - k0
                s1[t] = c if s1[t] is None else s1[t] + c
                s2[t] = c * c if s2[t] is None else s2[t] + c * c
        m1 = _bcast_rows_sum(s1[0] + s1[1]) * (1.0 / D)
        m2 = _bcast_rows_sum(s2[0] + s2[1]) * (1.0 / D)
        mean = k0 + m1
        rstd = jax.lax.rsqrt(jnp.maximum(m2 - m1 * m1, 0.0) + EPS)
        t1, t2 = [None, None], [None, None]
        for i in range(n16):
            p = x_s[8 * i:8 * i + 8, lt(j)]
            xs = []
            for t in range(2):
                xn = (_unpack2(p, t) - mean) * rstd
                xs.append(xn)
                t1[t] = xn if t1[t] is None else t1[t] + xn
                t2[t] = xn * xn if t2[t] is None else t2[t] + xn * xn
            xn_s[8 * i:8 * i + 8, lt(j)] = _pack(xs[0], xs[1])
        mean2 = _bcast_rows_sum(t1[0] + t1[1]) * (1.0 / D)
        e2 = _bcast_rows_sum(t2[0] + t2[1]) * (1.0 / D)
        rstd2 = jax.lax.rsqrt(jnp.maximum(e2 - mean2 * mean2, 0.0) + EPS)
        for i in range(n16):
            p = xn_s[8 * i:8 * i + 8, lt(j)]
            h_s[8 * i:8 * i + 8, lt(j)] = _pack((_unpack(p, 0) - mean2) * rstd2, (_unpack(p, 1) - mean2) * rstd2)
        return rstd2

    ST = 57

    def prep_wqkv(c, dep):
        rows = min(128, D - 128 * c)
        wp = wqkv_s[64 * c:64 * c + rows // 2, :]
        wp = jnp.where(jnp.tile(_never(dep), (rows // 16, 11))[:, :3 * D], jnp.uint32(0), wp)
        w = _as_bf16(wp).astype(f32)
        if rows < 128:
            w = jnp.concatenate([w, jnp.zeros((128 - rows, 3 * D), f32)], axis=0)
        wt = w.T
        for v in range(3 * D // 8):
            wt_f[c, pl.ds(8 * v + (8 * v) // 56, 8), :] = wt[8 * v:8 * v + 8]
        for sec in range(3):
            for d in range(DH):
                ev, od = (wt_f[c, pl.ds(sec * 8 * ST + DH * g + d, 8, stride=ST), :] for g in range(2))
                wt_s[c, sec * (D // 2) + 8 * d:sec * (D // 2) + 8 * d + 8, :] = _pack(ev, od)

    def prep_wo(c, dep):
        cols = min(128, D - 128 * c)
        wp = wo_s[:, 128 * c:128 * c + cols]
        wp = jnp.where(jnp.tile(_never(dep), (D // 16, 1))[:, :cols], jnp.uint32(0), wp)
        if cols < 128:
            wp = jnp.concatenate([wp, jnp.zeros((D // 2, 128 - cols), u32)], axis=1)
        wo_f[c] = wp
        parts = []
        for dp in range(DH // 2):
            gath = [wo_f[c, pl.ds(14 * 8 * g + dp, 8, stride=14), :] for g in range(2)]
            for e in range(2):
                parts.append(_pack(_unpack(gath[0], e), _unpack(gath[1], e)))
        wpk = _as_bf16(jnp.concatenate(parts, axis=0))
        wpk = jnp.concatenate([wpk, jnp.zeros((512 - D, 128), bf16)], axis=0)
        wpt = pltpu.bitcast(wpk.T, u32)
        rows = min(128, D - 128 * c) // 2
        for cc in range(4):
            wot_s[cc, 64 * c:64 * c + rows, :] = wpt[:rows, lt(cc)]

    def lhs_448(ref, r0, nr):
        rs = slice(r0 // 2, (r0 + nr) // 2)
        return jnp.concatenate([_as_bf16(ref[0, rs, :]), _as_bf16(ref[1, rs, :]), _as_bf16(ref[2, rs, :]),
                                _as_bf16(ref[3, rs, :])[:, 0:64]], axis=1)

    def qkv(j, sec):
        wt = lhs_448(wt_s, sec * D, D)
        res = jnp.dot(wt, _as_bf16(xn_s[:, lt(j)]), preferred_element_type=f32)
        if sec == 0:
            q_s[j] = res
        else:
            dst = k_s if sec == 1 else v_s
            for d in range(DH):
                dst[j, 8 * d:8 * d + 8, :] = _pack(res[16 * d:16 * d + 8], res[16 * d + 8:16 * d + 16])
        return res[0:8]

    def shifted(cur, prev, w):
        if w == 0:
            return cur
        sh = DIL * w
        return pltpu.roll(jnp.where(lane >= 128 - sh, prev, cur), sh, 1)

    def attention(j):
        jp = max(j - 1, 0)
        acc = [[None, None] for _ in range(W)]
        for d in range(DH):
            q = [q_s[j, 16 * d + 8 * g:16 * d + 8 * g + 8, :] for g in range(2)]
            k = k_s[j, 8 * d:8 * d + 8, :]
            kp = k_s[jp, 8 * d:8 * d + 8, :]
            for w in range(W):
                ks = shifted(k, kp, w)
                for g in range(2):
                    p = q[g] * _unpack(ks, g)
                    acc[w][g] = p if acc[w][g] is None else acc[w][g] + p
        scale = DH ** -0.5
        prob = [[None, None] for _ in range(W)]
        for g in range(2):
            lg = [acc[w][g] * scale for w in range(W)]
            if j == 0:
                lg = [lg[w] if w == 0 else jnp.where(lane >= DIL * w, lg[w], -1e9) for w in range(W)]
            m = lg[0]
            for w in range(1, W):
                m = jnp.maximum(m, lg[w])
            e = [jnp.exp(t - m) for t in lg]
            inv = 1.0 / _tree_sum(e)
            for w in range(W):
                prob[w][g] = e[w] * inv
        for d in range(DH):
            v = v_s[j, 8 * d:8 * d + 8, :]
            vp = v_s[jp, 8 * d:8 * d + 8, :]
            o = [None, None]
            for w in range(W):
                vs = shifted(v, vp, w)
                for g in range(2):
                    p = prob[w][g] * _unpack(vs, g)
                    o[g] = p if o[g] is None else o[g] + p
            o_s[j, 8 * d:8 * d + 8, :] = _pack(o[0], o[1])

    def oproj(j):
        wot = lhs_448(wot_s, 0, D)
        a = jnp.dot(wot, _as_bf16(o_s[j]), preferred_element_type=f32)
        b2 = b2_s[pl.ds(128 * j, 128)].astype(f32).reshape(1, 128)
        r_s[j] = a + _as_bf16(x_s[:, lt(j)]).astype(f32) + b2

    def mixer_up(b, c):
        hb = _as_bf16(h_s[:, lt(KB * b, KB)])
        wb = _as_bf16(w1_s[64 * KB * b:64 * KB * (b + 1), lt(c)])
        upd = jnp.dot(hb, wb, preferred_element_type=f32)
        if b == 0:
            u_s[:, lt(c)] = upd
        elif b < NB - 1:
            u_s[:, lt(c)] = u_s[:, lt(c)] + upd
        else:
            b1 = b1_s[pl.ds(128 * c, 128)].astype(f32).reshape(1, 128)
            t = u_s[:, lt(c)] + upd + b1
            ub_s[:, lt(c)] = pltpu.bitcast(jax.nn.gelu(t, approximate=True).astype(bf16), u32)
        return upd[0:8]

    def mixer_down(j0, nj):
        ub = _as_bf16(ub_s[...])
        if isinstance(j0, int):
            cols = lambda t, n: lt(j0 + t, n)
        else:
            cols = lambda t, n: pl.ds(pl.multiple_of((j0 + t) * 128, 128), 128 * n)
        y = jnp.dot(ub, _as_bf16(w2_s[:, cols(0, nj)]), preferred_element_type=f32)
        for t in range(nj):
            out_s[:, cols(t, 1)] = pltpu.bitcast((y[:, lt(t)] + r_s[j0 + t]).astype(bf16), u32)

    def tiles(b):
        return range(KB * b, KB * b + KB)

    tok = None
    for j in tiles(0):
        cp_xt[j].wait(tok)
        tok = layer_norms(j)
    for c in range(NF):
        if c % 2 == 0:
            cp_w10[c // 2].wait(tok)
        tok = mixer_up(0, c)
        for i in range(4):
            if PREP_AT[i] == c:
                cp_wqkv[i].wait(tok)
                prep_wqkv(i, tok)

    def out_copy(j0, n, sem):
        if isinstance(j0, int):
            sl = lt(j0, n)
        else:
            sl = pl.ds(pl.multiple_of(j0 * 128, 128), 128 * n)
        return pltpu.make_async_copy(out_s.at[:, sl], out_hbm.at[:, sl], sems.at[sem])

    for b in range(NB):
        for t, j in enumerate(tiles(b)):
            for sec in range(3):
                tok = qkv(j, sec)
                if b == 0 and t == 0 and sec == 0:
                    cp_x1.wait(tok)
                if b == 0 and 3 * t + sec in LNQ_AT:
                    layer_norms(KB + LNQ_AT.index(3 * t + sec), tok)
                if t == KB - 1 and sec == 1:
                    if b + 1 < NB:
                        cp_w1[b + 1].wait(tok)
                    else:
                        for c in cp_w2:
                            c.wait(tok)
            attention(j)
        if b + 1 < NB:
            ln_at = dict(zip(LN_AT, tiles(b + 2))) if b + 2 < NB else {}
            for c in range(NF):
                tok = mixer_up(b + 1, c)
                if b == 0:
                    if c == 2:
                        cp_wo.wait(tok)
                        cp_b2.wait(tok)
                    if c == 4:
                        cp_x2.wait(tok)
                    if c in PREP_WO_AT:
                        prep_wo(PREP_WO_AT.index(c), tok)
                if b == 1 and c == 2:
                    cp_x3.wait(tok)
                    cp_b1.wait(tok)
                if c in ln_at:
                    layer_norms(ln_at[c], tok)
            for j in tiles(b):
                oproj(j)
        else:
            mixer_down(0, 2)
            for j in tiles(b):
                oproj(j)
    s0 = sem_i[0]
    out_copy(0, 2, s0).start()

    def body(i, carry):
        j0 = 2 + 2 * LOOP_P * i
        for p in range(LOOP_P):
            mixer_down(j0 + 2 * p, 2)
        out_copy(j0, 2 * LOOP_P, s0 + 1 + i).start()
        return carry

    jax.lax.fori_loop(0, LOOP_N, body, 0)
    jt = 2 + 2 * LOOP_P * LOOP_N
    for j0 in range(jt, NT, 2):
        mixer_down(j0, 2)
    out_copy(jt, NT - jt, s0 + 1 + LOOP_N).start()
    out_copy(0, 2, s0).wait()
    for i in range(LOOP_N):
        out_copy(2 + 2 * LOOP_P * i, 2 * LOOP_P, s0 + 1 + i).wait()
    out_copy(jt, NT - jt, s0 + 1 + LOOP_N).wait()


@jax.jit
def pallas_parallel_sum__sliding_local_dilated__mixer_token_mlp__prompt_kernel(
    A_x, A_wqkv, A_wo, B_x, B_w1, B_b1, B_w2, B_b2,
):
    del B_x
    xT = A_x.reshape(S, D).T
    any_spec = pl.BlockSpec(memory_space=pl.ANY)
    scratch = [
        pltpu.VMEM((D // 2, S), u32),
        pltpu.VMEM((D // 2, 3 * D), u32),
        pltpu.VMEM((D // 2, D), u32),
        pltpu.VMEM((S // 2, F), u32),
        pltpu.VMEM((F // 2, S), u32),
        pltpu.VMEM((F,), bf16),
        pltpu.VMEM((S,), bf16),
        pltpu.VMEM((4, 24 * 57, 128), f32),
        pltpu.VMEM((4, D // 2, 128), u32),
        pltpu.VMEM((4, 3 * D // 2, 128), u32),
        pltpu.VMEM((4, D // 2, 128), u32),
        pltpu.VMEM((D // 2, S), u32),
        pltpu.VMEM((D // 2, S), u32),
        pltpu.VMEM((NT, D, 128), f32),
        pltpu.VMEM((NT, D // 2, 128), u32),
        pltpu.VMEM((NT, D // 2, 128), u32),
        pltpu.VMEM((NT, D, 128), u32),
        pltpu.VMEM((NT, D, 128), f32),
        pltpu.VMEM((D, F), f32),
        pltpu.VMEM((D // 2, F), u32),
        pltpu.VMEM((D // 2, S), u32),
        pltpu.SemaphoreType.DMA((N_SEMS,)),
    ]
    scratch[16] = pltpu.VMEM((NT, D // 2, 128), u32)
    outT = pl.pallas_call(
        _kernel,
        out_shape=jax.ShapeDtypeStruct((D, S), bf16),
        in_specs=[any_spec] * 7,
        out_specs=any_spec,
        scratch_shapes=scratch,
        compiler_params=pltpu.CompilerParams(vmem_limit_bytes=100 * 1024 * 1024, flags=FLAGS),
        name="fused_kernel",
    )(xT, A_wqkv, A_wo, B_w1, B_b1, B_w2, B_b2)
    return outT.T.reshape(1, S, D)
```

```python
import jax
import jax.numpy as jnp
import numpy as np
import jax.experimental.pallas as pl
import jax.experimental.pallas.tpu as pltpu

S, D, H, DH, F = 2048, 448, 16, 28, 1792
W, DIL = 8, 2
NT = S // 128
NF = F // 128
EPS = 1e-5
f32, bf16, u32, i32 = jnp.float32, jnp.bfloat16, jnp.uint32, jnp.int32


def _unpack(x, i):
    return pltpu.unpack_elementwise(x, index=i, packed_dtype=bf16, unpacked_dtype=f32)


def _unpack2(x, i):
    if i == 0:
        return jax.lax.bitcast_convert_type(x << 16, f32)
    return jax.lax.bitcast_convert_type(x & jnp.uint32(0xFFFF0000), f32)


def _pack(a, b):
    return pltpu.pack_elementwise([a, b], packed_dtype=bf16)


def _as_bf16(x_u32):
    return pltpu.bitcast(x_u32, bf16)


def _tree_sum(xs):
    xs = list(xs)
    while len(xs) > 1:
        nxt = [xs[i] + xs[i + 1] for i in range(0, len(xs) - 1, 2)]
        if len(xs) % 2:
            nxt.append(xs[-1])
        xs = nxt
    return xs[0]


def _bcast_rows_sum(p):
    t = jnp.sum(p, axis=0, keepdims=True)
    return jnp.broadcast_to(t, (8, 128))


def _never(tok):
    return tok * tok < -1.0


def _zero_after(tok):
    return jnp.where(_never(tok), 1.0, 0.0).astype(f32)


KB = 4
NB = NT // KB
LOOP_N, LOOP_P = (2, 3)
QONE = 1
SMX = 1
DMA_AFTER_C = {0: ('x2',), 1: ('q',), 3: ('q',), 5: ('q',), 6: ('q', 'wo')}
KSPLIT = 1
LN_A_AT = {4: 7, 5: 9, 6: 11, 7: 12, 8: 14, 9: 18, 10: 22, 11: 25}
LN_B_AT = {12: (0, 4), 13: (0, 6), 14: (1, 4), 15: (1, 6)}
PREP_AT = (16, 20, 24, 26)
PREP_WO_AT = (0, 1, 2, 3)
FLAGS = {"XLA_TPU_RESCHEDULE_DMA_DONES": True, "XLA_TPU_EVENLY_DISTRIBUTE_CRITICAL_NODES": True}
N_SEMS = 64


def _kernel(x_hbm, wqkv_hbm, wo_hbm, w1_hbm, b1_hbm, w2_hbm, b2_hbm, out_hbm,
            x_s, wqkv_s, wo_s, w1_s, w2_s, b1_s, b2_s,
            wt_f, wo_f, wt_s, wot_s,
            xn_s, h_s, q_s, k_s, v_s, o_s, r_s, u_s, ub_s, out_s, sems):
    x_hbm, wqkv_hbm, wo_hbm, w1_hbm, w2_hbm, out_hbm = (
        r.bitcast(u32) for r in (x_hbm, wqkv_hbm, wo_hbm, w1_hbm, w2_hbm, out_hbm))
    sem_i = [0]

    class Dma:
        def __init__(self, src, dst):
            self.src, self.dst, self.i = src, dst, sem_i[0]
            sem_i[0] += 1
            pltpu.make_async_copy(src, dst, sems.at[self.i]).start()

        def wait(self, tok=None):
            idx = self.i
            if tok is not None:
                idx = idx + jnp.where(_never(tok), 1, 0).astype(i32)[0, 0]
            pltpu.make_async_copy(self.src, self.dst, sems.at[idx]).wait()

    def lt(j, n=1):
        return slice(128 * j, 128 * (j + n))

    def x_dma(j, n):
        return Dma(x_hbm.at[:, lt(j, n)], x_s.at[:, lt(j, n)])

    def w1_dma(t0, nt, c0=0, n=NF):
        rows = pl.ds(64 * t0, 64 * nt)
        return Dma(w1_hbm.at[rows, lt(c0, n)], w1_s.at[rows, lt(c0, n)])

    def wqkv_dma(c):
        rows = pl.ds(64 * c, min(64, D // 2 - 64 * c))
        return Dma(wqkv_hbm.at[rows], wqkv_s.at[rows])

    if KSPLIT:
        start = [(0, 2, 2 * i, 2) for i in range(NF // 2)] + [(2, 2, 2 * i, 2) for i in range(NF // 2)]
    else:
        start = [(0, 4, c, 1) for c in range(NF)]
    start += [(4, 4, c, 1) for c in range(NF)]

    cp_x = {}
    cp_start = {}
    cp_wqkv = []
    if KSPLIT:
        cp_x[0] = x_dma(0, 1)
        cp_x[1] = x_dma(1, 1)
        for i in range(NF // 2):
            cp_start[i] = w1_dma(0, 2, 2 * i, 2)
            if i in (1, 2):
                cp_x[i + 1] = x_dma(i + 1, 1)
        for i in range(NF // 2):
            cp_start[NF // 2 + i] = w1_dma(2, 2, 2 * i, 2)
            if i == 1:
                cp_x1 = x_dma(KB, KB)
    else:
        for j in range(KB):
            cp_x[j] = x_dma(j, 1)
        for i in range(NF // 2):
            cp_start[2 * i] = w1_dma(0, 4, 2 * i, 2)
            if i == 2:
                cp_x1 = x_dma(KB, KB)
    for i in range(NF // 2):
        cp_start[NF + 2 * i] = w1_dma(4, 4, 2 * i, 2)
        for extra in DMA_AFTER_C.get(i, ()):
            if extra == "x2":
                cp_x2 = x_dma(2 * KB, KB)
            elif extra == "wo":
                cp_wo = Dma(wo_hbm, wo_s)
                cp_b2 = Dma(b2_hbm, b2_s)
            else:
                cp_wqkv.append(wqkv_dma(len(cp_wqkv)))
    cp_x3 = x_dma(3 * KB, KB)
    cp_b1 = Dma(b1_hbm, b1_s)
    cp_w1 = {(b, hf): w1_dma(KB * (2 + b), KB, 7 * hf, 7) for b in range(2) for hf in range(2)}
    cp_w2 = [Dma(w2_hbm.at[:, lt(4 * b, 4)], w2_s.at[:, lt(4 * b, 4)]) for b in range(4)]

    lane = jax.lax.broadcasted_iota(jnp.int32, (8, 128), 1)

    def layer_norms(j, dep=None):
        n16 = D // 16
        k0 = jnp.broadcast_to(_unpack(x_s[0:8, lt(j)], 0)[0:1, :], (8, 128))
        if dep is not None:
            k0 = k0 + _zero_after(dep)
        s1, s2 = [None, None], [None, None]
        for i in range(n16):
            p = x_s[8 * i:8 * i + 8, lt(j)]
            for t in range(2):
                c = _unpack(p, t) - k0
                s1[t] = c if s1[t] is None else s1[t] + c
                s2[t] = c * c if s2[t] is None else s2[t] + c * c
        m1 = _bcast_rows_sum(s1[0] + s1[1]) * (1.0 / D)
        m2 = _bcast_rows_sum(s2[0] + s2[1]) * (1.0 / D)
        mean = k0 + m1
        rstd = jax.lax.rsqrt(jnp.maximum(m2 - m1 * m1, 0.0) + EPS)
        t1, t2 = [None, None], [None, None]
        for i in range(n16):
            p = x_s[8 * i:8 * i + 8, lt(j)]
            xs = []
            for t in range(2):
                xn = (_unpack2(p, t) - mean) * rstd
                xs.append(xn)
                t1[t] = xn if t1[t] is None else t1[t] + xn
                t2[t] = xn * xn if t2[t] is None else t2[t] + xn * xn
            xn_s[8 * i:8 * i + 8, lt(j)] = _pack(xs[0], xs[1])
        mean2 = _bcast_rows_sum(t1[0] + t1[1]) * (1.0 / D)
        e2 = _bcast_rows_sum(t2[0] + t2[1]) * (1.0 / D)
        rstd2 = jax.lax.rsqrt(jnp.maximum(e2 - mean2 * mean2, 0.0) + EPS)
        for i in range(n16):
            p = xn_s[8 * i:8 * i + 8, lt(j)]
            h_s[8 * i:8 * i + 8, lt(j)] = _pack((_unpack(p, 0) - mean2) * rstd2, (_unpack(p, 1) - mean2) * rstd2)
        return rstd2

    ST = 57

    def prep_wqkv(c, dep):
        rows = min(128, D - 128 * c)
        wp = wqkv_s[64 * c:64 * c + rows // 2, :]
        wp = jnp.where(jnp.tile(_never(dep), (rows // 16, 11))[:, :3 * D], jnp.uint32(0), wp)
        w = _as_bf16(wp).astype(f32)
        if rows < 128:
            w = jnp.concatenate([w, jnp.zeros((128 - rows, 3 * D), f32)], axis=0)
        wt = w.T
        for v in range(3 * D // 8):
            wt_f[c, pl.ds(8 * v + (8 * v) // 56, 8), :] = wt[8 * v:8 * v + 8]
        for sec in range(3):
            for d in range(DH):
                ev, od = (wt_f[c, pl.ds(sec * 8 * ST + DH * g + d, 8, stride=ST), :] for g in range(2))
                wt_s[c, sec * (D // 2) + 8 * d:sec * (D // 2) + 8 * d + 8, :] = _pack(ev, od)

    def prep_wo(c, dep):
        cols = min(128, D - 128 * c)
        wp = wo_s[:, 128 * c:128 * c + cols]
        wp = jnp.where(jnp.tile(_never(dep), (D // 16, 1))[:, :cols], jnp.uint32(0), wp)
        if cols < 128:
            wp = jnp.concatenate([wp, jnp.zeros((D // 2, 128 - cols), u32)], axis=1)
        wo_f[c] = wp
        parts = []
        for dp in range(DH // 2):
            gath = [wo_f[c, pl.ds(14 * 8 * g + dp, 8, stride=14), :] for g in range(2)]
            for e in range(2):
                parts.append(_pack(_unpack(gath[0], e), _unpack(gath[1], e)))
        wpk = _as_bf16(jnp.concatenate(parts, axis=0))
        wpk = jnp.concatenate([wpk, jnp.zeros((512 - D, 128), bf16)], axis=0)
        wpt = pltpu.bitcast(wpk.T, u32)
        rows = min(128, D - 128 * c) // 2
        for cc in range(4):
            wot_s[cc, 64 * c:64 * c + rows, :] = wpt[:rows, lt(cc)]

    def lhs_448(ref, r0, nr):
        rs = slice(r0 // 2, (r0 + nr) // 2)
        return jnp.concatenate([_as_bf16(ref[0, rs, :]), _as_bf16(ref[1, rs, :]), _as_bf16(ref[2, rs, :]),
                                _as_bf16(ref[3, rs, :])[:, 0:64]], axis=1)

    def qkv_store(j, sec, res):
        if sec == 0:
            q_s[j] = res
        else:
            dst = k_s if sec == 1 else v_s
            for d in range(DH):
                dst[j, 8 * d:8 * d + 8, :] = _pack(res[16 * d:16 * d + 8], res[16 * d + 8:16 * d + 16])

    def qkv(j, sec):
        if QONE:
            if sec == 0:
                wt = lhs_448(wt_s, 0, 3 * D)
                res = jnp.dot(wt, _as_bf16(xn_s[:, lt(j)]), preferred_element_type=f32)
                for s3 in range(3):
                    qkv_store(j, s3, res[s3 * D:(s3 + 1) * D])
                qkv.res = res
            return qkv.res[sec * D:sec * D + 8]
        wt = lhs_448(wt_s, sec * D, D)
        res = jnp.dot(wt, _as_bf16(xn_s[:, lt(j)]), preferred_element_type=f32)
        qkv_store(j, sec, res)
        return res[0:8]

    def shifted(cur, prev, w):
        if w == 0:
            return cur
        sh = DIL * w
        return pltpu.roll(jnp.where(lane >= 128 - sh, prev, cur), sh, 1)

    def attention(j):
        jp = max(j - 1, 0)
        acc = [[None, None] for _ in range(W)]
        for d in range(DH):
            q = [q_s[j, 16 * d + 8 * g:16 * d + 8 * g + 8, :] for g in range(2)]
            k = k_s[j, 8 * d:8 * d + 8, :]
            kp = k_s[jp, 8 * d:8 * d + 8, :]
            for w in range(W):
                ks = shifted(k, kp, w)
                for g in range(2):
                    p = q[g] * _unpack(ks, g)
                    acc[w][g] = p if acc[w][g] is None else acc[w][g] + p
        scale = DH ** -0.5
        prob = [[None, None] for _ in range(W)]
        for g in range(2):
            if SMX:
                lg = [acc[w][g] for w in range(W)]
                if j == 0:
                    lg = [lg[w] if w == 0 else jnp.where(lane >= DIL * w, lg[w], -1e9 / scale) for w in range(W)]
                m = lg[0]
                for w in range(1, W):
                    m = jnp.maximum(m, lg[w])
                e = [jnp.exp2((t - m) * (scale * 1.4426950408889634)) for t in lg]
            else:
                lg = [acc[w][g] * scale for w in range(W)]
                if j == 0:
                    lg = [lg[w] if w == 0 else jnp.where(lane >= DIL * w, lg[w], -1e9) for w in range(W)]
                m = lg[0]
                for w in range(1, W):
                    m = jnp.maximum(m, lg[w])
                e = [jnp.exp(t - m) for t in lg]
            inv = 1.0 / _tree_sum(e)
            for w in range(W):
                prob[w][g] = e[w] * inv
        for d in range(DH):
            v = v_s[j, 8 * d:8 * d + 8, :]
            vp = v_s[jp, 8 * d:8 * d + 8, :]
            o = [None, None]
            for w in range(W):
                vs = shifted(v, vp, w)
                for g in range(2):
                    p = prob[w][g] * _unpack(vs, g)
                    o[g] = p if o[g] is None else o[g] + p
            o_s[j, 8 * d:8 * d + 8, :] = _pack(o[0], o[1])

    def oproj(j):
        wot = lhs_448(wot_s, 0, D)
        a = jnp.dot(wot, _as_bf16(o_s[j]), preferred_element_type=f32)
        b2 = b2_s[pl.ds(128 * j, 128)].astype(f32).reshape(1, 128)
        r_s[j] = a + _as_bf16(x_s[:, lt(j)]).astype(f32) + b2

    def mixer_up(t0, nt, c0, nc):
        hb = _as_bf16(h_s[:, lt(t0, nt)])
        wb = _as_bf16(w1_s[64 * t0:64 * (t0 + nt), lt(c0, nc)])
        upd = jnp.dot(hb, wb, preferred_element_type=f32)
        if t0 == 0:
            u_s[:, lt(c0, nc)] = upd
        elif t0 + nt < NT:
            u_s[:, lt(c0, nc)] = u_s[:, lt(c0, nc)] + upd
        else:
            b1 = b1_s[pl.ds(128 * c0, 128 * nc)].astype(f32).reshape(1, 128 * nc)
            t = u_s[:, lt(c0, nc)] + upd + b1
            ub_s[:, lt(c0, nc)] = pltpu.bitcast(jax.nn.gelu(t, approximate=True).astype(bf16), u32)
        return upd[0:8, 0:128]

    def mixer_down(j0, nj):
        ub = _as_bf16(ub_s[...])
        if isinstance(j0, int):
            cols = lambda t, n: lt(j0 + t, n)
        else:
            cols = lambda t, n: pl.ds(pl.multiple_of((j0 + t) * 128, 128), 128 * n)
        y = jnp.dot(ub, _as_bf16(w2_s[:, cols(0, nj)]), preferred_element_type=f32)
        for t in range(nj):
            out_s[:, cols(t, 1)] = pltpu.bitcast((y[:, lt(t)] + r_s[j0 + t]).astype(bf16), u32)

    def tiles(b):
        return range(KB * b, KB * b + KB)

    tok = None
    n_first = 2 if KSPLIT else KB
    for j in range(n_first):
        cp_x[j].wait(tok)
        tok = layer_norms(j)
    ln_at = {}
    for j, p in LN_A_AT.items():
        ln_at.setdefault(p, []).append(j)
    for p, piece in enumerate(start):
        if p in cp_start:
            cp_start[p].wait(tok)
        tok = mixer_up(*piece)
        if KSPLIT and p in (1, 2):
            cp_x[p + 1].wait(tok)
            layer_norms(p + 1, tok)
        if p == min(LN_A_AT[j] for j in range(KB, 2 * KB)):
            cp_x1.wait(tok)
        if p == min(LN_A_AT[j] for j in range(2 * KB, 3 * KB)):
            cp_x2.wait(tok)
        for i in range(4):
            if PREP_AT[i] == p:
                cp_wqkv[i].wait(tok)
                prep_wqkv(i, tok)
        for j in ln_at.get(p, ()):
            layer_norms(j, tok)

    def out_copy(j0, n, sem):
        if isinstance(j0, int):
            sl = lt(j0, n)
        else:
            sl = pl.ds(pl.multiple_of(j0 * 128, 128), 128 * n)
        return pltpu.make_async_copy(out_s.at[:, sl], out_hbm.at[:, sl], sems.at[sem])

    for b in range(NB):
        kb, hf = b // 2, b % 2
        for t, j in enumerate(tiles(b)):
            for sec in range(3):
                tok = qkv(j, sec)
                if b == 0:
                    for i in range(4):
                        if PREP_WO_AT[i] == 3 * t + sec:
                            if i == 0:
                                cp_wo.wait(tok)
                                cp_b2.wait(tok)
                            prep_wo(i, tok)
                if t == KB - 1 and sec == 1:
                    cp_w1[kb, hf].wait(tok)
                    if b == 0:
                        cp_x3.wait(tok)
                    if b == 2:
                        cp_b1.wait(tok)
                    if b == NB - 1:
                        for c in cp_w2:
                            c.wait(tok)
            attention(j)
        for i in range(7):
            tok = mixer_up(KB * (2 + kb), KB, 7 * hf + i, 1)
            for j, at in LN_B_AT.items():
                if at == (b, i):
                    layer_norms(j, tok)
        for j in tiles(b):
            oproj(j)
    mixer_down(0, 2)
    s0 = sem_i[0]
    out_copy(0, 2, s0).start()

    def body(i, carry):
        j0 = 2 + 2 * LOOP_P * i
        for p in range(LOOP_P):
            mixer_down(j0 + 2 * p, 2)
        out_copy(j0, 2 * LOOP_P, s0 + 1 + i).start()
        return carry

    jax.lax.fori_loop(0, LOOP_N, body, 0)
    jt = 2 + 2 * LOOP_P * LOOP_N
    for j0 in range(jt, NT, 2):
        mixer_down(j0, 2)
    out_copy(jt, NT - jt, s0 + 1 + LOOP_N).start()
    out_copy(0, 2, s0).wait()
    for i in range(LOOP_N):
        out_copy(2 + 2 * LOOP_P * i, 2 * LOOP_P, s0 + 1 + i).wait()
    out_copy(jt, NT - jt, s0 + 1 + LOOP_N).wait()


@jax.jit
def pallas_parallel_sum__sliding_local_dilated__mixer_token_mlp__prompt_kernel(
    A_x, A_wqkv, A_wo, B_x, B_w1, B_b1, B_w2, B_b2,
):
    del B_x
    xT = A_x.reshape(S, D).T
    any_spec = pl.BlockSpec(memory_space=pl.ANY)
    scratch = [
        pltpu.VMEM((D // 2, S), u32),
        pltpu.VMEM((D // 2, 3 * D), u32),
        pltpu.VMEM((D // 2, D), u32),
        pltpu.VMEM((S // 2, F), u32),
        pltpu.VMEM((F // 2, S), u32),
        pltpu.VMEM((F,), bf16),
        pltpu.VMEM((S,), bf16),
        pltpu.VMEM((4, 24 * 57, 128), f32),
        pltpu.VMEM((4, D // 2, 128), u32),
        pltpu.VMEM((4, 3 * D // 2, 128), u32),
        pltpu.VMEM((4, D // 2, 128), u32),
        pltpu.VMEM((D // 2, S), u32),
        pltpu.VMEM((D // 2, S), u32),
        pltpu.VMEM((NT, D, 128), f32),
        pltpu.VMEM((NT, D // 2, 128), u32),
        pltpu.VMEM((NT, D // 2, 128), u32),
        pltpu.VMEM((NT, D, 128), u32),
        pltpu.VMEM((NT, D, 128), f32),
        pltpu.VMEM((D, F), f32),
        pltpu.VMEM((D // 2, F), u32),
        pltpu.VMEM((D // 2, S), u32),
        pltpu.SemaphoreType.DMA((N_SEMS,)),
    ]
    scratch[16] = pltpu.VMEM((NT, D // 2, 128), u32)
    outT = pl.pallas_call(
        _kernel,
        out_shape=jax.ShapeDtypeStruct((D, S), bf16),
        in_specs=[any_spec] * 7,
        out_specs=any_spec,
        scratch_shapes=scratch,
        compiler_params=pltpu.CompilerParams(vmem_limit_bytes=100 * 1024 * 1024, flags=FLAGS),
        name="fused_kernel",
    )(xT, A_wqkv, A_wo, B_w1, B_b1, B_w2, B_b2)
    return outT.T.reshape(1, S, D)
```

```python
import jax
import jax.numpy as jnp
import numpy as np
import jax.experimental.pallas as pl
import jax.experimental.pallas.tpu as pltpu

S, D, H, DH, F = 2048, 448, 16, 28, 1792
W, DIL = 8, 2
NT = S // 128
NF = F // 128
EPS = 1e-5
f32, bf16, u32, i32 = jnp.float32, jnp.bfloat16, jnp.uint32, jnp.int32


def _unpack(x, i):
    return pltpu.unpack_elementwise(x, index=i, packed_dtype=bf16, unpacked_dtype=f32)


def _unpack2(x, i):
    if i == 0:
        return jax.lax.bitcast_convert_type(x << 16, f32)
    return jax.lax.bitcast_convert_type(x & jnp.uint32(0xFFFF0000), f32)


def _pack(a, b):
    return pltpu.pack_elementwise([a, b], packed_dtype=bf16)


def _as_bf16(x_u32):
    return pltpu.bitcast(x_u32, bf16)


def _tree_sum(xs):
    xs = list(xs)
    while len(xs) > 1:
        nxt = [xs[i] + xs[i + 1] for i in range(0, len(xs) - 1, 2)]
        if len(xs) % 2:
            nxt.append(xs[-1])
        xs = nxt
    return xs[0]


def _bcast_rows_sum(p):
    t = jnp.sum(p, axis=0, keepdims=True)
    return jnp.broadcast_to(t, (8, 128))


def _never(tok):
    return tok * tok < -1.0


def _zero_after(tok):
    return jnp.where(_never(tok), 1.0, 0.0).astype(f32)


KB = 4
NB = NT // KB
LOOP_N, LOOP_P = (2, 3)
QONE = 1
SMX = 1
DMA_AFTER_C = {0: ('x2',), 1: ('q',), 3: ('q',), 5: ('q',), 6: ('q', 'wo')}
X23_AFTER = (5, 6)
LN23_AT = (4, 5)
NACC = 2
KSPLIT = 1
LN_A_AT = {4: 7, 5: 9, 6: 11, 7: 12, 8: 14, 9: 15, 10: 18, 11: 22}
LN_B_AT = {12: (0, 4), 13: (0, 6), 14: (1, 4), 15: (1, 6)}
PREP_AT = (16, 20, 24, 26)
PREP_WO_AT = (0, 1, 2, 3)
FLAGS = {"XLA_TPU_RESCHEDULE_DMA_DONES": True, "XLA_TPU_EVENLY_DISTRIBUTE_CRITICAL_NODES": True}
N_SEMS = 64


def _kernel(x_hbm, wqkv_hbm, wo_hbm, w1_hbm, b1_hbm, w2_hbm, b2_hbm, out_hbm,
            x_s, wqkv_s, wo_s, w1_s, w2_s, b1_s, b2_s,
            wt_f, wo_f, wt_s, wot_s,
            xn_s, h_s, q_s, k_s, v_s, o_s, r_s, u_s, ub_s, out_s, sems):
    x_hbm, wqkv_hbm, wo_hbm, w1_hbm, w2_hbm, out_hbm = (
        r.bitcast(u32) for r in (x_hbm, wqkv_hbm, wo_hbm, w1_hbm, w2_hbm, out_hbm))
    sem_i = [0]

    class Dma:
        def __init__(self, src, dst):
            self.src, self.dst, self.i = src, dst, sem_i[0]
            sem_i[0] += 1
            pltpu.make_async_copy(src, dst, sems.at[self.i]).start()

        def wait(self, tok=None):
            idx = self.i
            if tok is not None:
                idx = idx + jnp.where(_never(tok), 1, 0).astype(i32)[0, 0]
            pltpu.make_async_copy(self.src, self.dst, sems.at[idx]).wait()

    def lt(j, n=1):
        return slice(128 * j, 128 * (j + n))

    def x_dma(j, n):
        return Dma(x_hbm.at[:, lt(j, n)], x_s.at[:, lt(j, n)])

    def w1_dma(t0, nt, c0=0, n=NF):
        rows = pl.ds(64 * t0, 64 * nt)
        return Dma(w1_hbm.at[rows, lt(c0, n)], w1_s.at[rows, lt(c0, n)])

    def wqkv_dma(c):
        rows = pl.ds(64 * c, min(64, D // 2 - 64 * c))
        return Dma(wqkv_hbm.at[rows], wqkv_s.at[rows])

    if KSPLIT:
        start = [(0, 2, 2 * i, 2) for i in range(NF // 2)] + [(2, 2, 2 * i, 2) for i in range(NF // 2)]
    else:
        start = [(0, 4, c, 1) for c in range(NF)]
    start += [(4, 4, c, 1) for c in range(NF)]

    cp_x = {}
    cp_start = {}
    cp_wqkv = []
    if KSPLIT:
        cp_x[0] = x_dma(0, 1)
        cp_x[1] = x_dma(1, 1)
        for i in range(NF // 2):
            cp_start[i] = w1_dma(0, 2, 2 * i, 2)
            if i in X23_AFTER:
                jx = 2 + X23_AFTER.index(i)
                cp_x[jx] = x_dma(jx, 1)
        for i in range(NF // 2):
            cp_start[NF // 2 + i] = w1_dma(2, 2, 2 * i, 2)
            if i == 1:
                cp_x1 = x_dma(KB, KB)
    else:
        for j in range(KB):
            cp_x[j] = x_dma(j, 1)
        for i in range(NF // 2):
            cp_start[2 * i] = w1_dma(0, 4, 2 * i, 2)
            if i == 2:
                cp_x1 = x_dma(KB, KB)
    for i in range(NF // 2):
        cp_start[NF + 2 * i] = w1_dma(4, 4, 2 * i, 2)
        for extra in DMA_AFTER_C.get(i, ()):
            if extra == "x2":
                cp_x2 = x_dma(2 * KB, KB)
            elif extra == "wo":
                cp_wo = Dma(wo_hbm, wo_s)
                cp_b2 = Dma(b2_hbm, b2_s)
            else:
                cp_wqkv.append(wqkv_dma(len(cp_wqkv)))
    cp_x3 = x_dma(3 * KB, KB)
    cp_b1 = Dma(b1_hbm, b1_s)
    cp_w1 = {(b, hf): w1_dma(KB * (2 + b), KB, 7 * hf, 7) for b in range(2) for hf in range(2)}
    cp_w2 = [Dma(w2_hbm.at[:, lt(4 * b, 4)], w2_s.at[:, lt(4 * b, 4)]) for b in range(4)]

    lane = jax.lax.broadcasted_iota(jnp.int32, (8, 128), 1)

    def layer_norms(j, dep=None):
        n16 = D // 16
        k0 = jnp.broadcast_to(_unpack(x_s[0:8, lt(j)], 0)[0:1, :], (8, 128))
        if dep is not None:
            k0 = k0 + _zero_after(dep)
        s1, s2 = [None, None], [None, None]
        for i in range(n16):
            p = x_s[8 * i:8 * i + 8, lt(j)]
            for t in range(2):
                c = _unpack(p, t) - k0
                a = t % NACC
                s1[a] = c if s1[a] is None else s1[a] + c
                s2[a] = c * c if s2[a] is None else s2[a] + c * c
        m1 = _bcast_rows_sum(sum(s1[1:NACC], s1[0])) * (1.0 / D)
        m2 = _bcast_rows_sum(sum(s2[1:NACC], s2[0])) * (1.0 / D)
        mean = k0 + m1
        rstd = jax.lax.rsqrt(jnp.maximum(m2 - m1 * m1, 0.0) + EPS)
        t1, t2 = [None, None], [None, None]
        for i in range(n16):
            p = x_s[8 * i:8 * i + 8, lt(j)]
            xs = []
            for t in range(2):
                xn = (_unpack2(p, t) - mean) * rstd
                xs.append(xn)
                a = t % NACC
                t1[a] = xn if t1[a] is None else t1[a] + xn
                t2[a] = xn * xn if t2[a] is None else t2[a] + xn * xn
            xn_s[8 * i:8 * i + 8, lt(j)] = _pack(xs[0], xs[1])
        mean2 = _bcast_rows_sum(sum(t1[1:NACC], t1[0])) * (1.0 / D)
        e2 = _bcast_rows_sum(sum(t2[1:NACC], t2[0])) * (1.0 / D)
        rstd2 = jax.lax.rsqrt(jnp.maximum(e2 - mean2 * mean2, 0.0) + EPS)
        for i in range(n16):
            p = xn_s[8 * i:8 * i + 8, lt(j)]
            h_s[8 * i:8 * i + 8, lt(j)] = _pack((_unpack(p, 0) - mean2) * rstd2, (_unpack(p, 1) - mean2) * rstd2)
        return rstd2

    ST = 57

    def prep_wqkv(c, dep):
        rows = min(128, D - 128 * c)
        wp = wqkv_s[64 * c:64 * c + rows // 2, :]
        wp = jnp.where(jnp.tile(_never(dep), (rows // 16, 11))[:, :3 * D], jnp.uint32(0), wp)
        w = _as_bf16(wp).astype(f32)
        if rows < 128:
            w = jnp.concatenate([w, jnp.zeros((128 - rows, 3 * D), f32)], axis=0)
        wt = w.T
        for v in range(3 * D // 8):
            wt_f[c, pl.ds(8 * v + (8 * v) // 56, 8), :] = wt[8 * v:8 * v + 8]
        for sec in range(3):
            for d in range(DH):
                ev, od = (wt_f[c, pl.ds(sec * 8 * ST + DH * g + d, 8, stride=ST), :] for g in range(2))
                wt_s[c, sec * (D // 2) + 8 * d:sec * (D // 2) + 8 * d + 8, :] = _pack(ev, od)

    def prep_wo(c, dep):
        cols = min(128, D - 128 * c)
        wp = wo_s[:, 128 * c:128 * c + cols]
        wp = jnp.where(jnp.tile(_never(dep), (D // 16, 1))[:, :cols], jnp.uint32(0), wp)
        if cols < 128:
            wp = jnp.concatenate([wp, jnp.zeros((D // 2, 128 - cols), u32)], axis=1)
        wo_f[c] = wp
        parts = []
        for dp in range(DH // 2):
            gath = [wo_f[c, pl.ds(14 * 8 * g + dp, 8, stride=14), :] for g in range(2)]
            for e in range(2):
                parts.append(_pack(_unpack(gath[0], e), _unpack(gath[1], e)))
        wpk = _as_bf16(jnp.concatenate(parts, axis=0))
        wpk = jnp.concatenate([wpk, jnp.zeros((512 - D, 128), bf16)], axis=0)
        wpt = pltpu.bitcast(wpk.T, u32)
        rows = min(128, D - 128 * c) // 2
        for cc in range(4):
            wot_s[cc, 64 * c:64 * c + rows, :] = wpt[:rows, lt(cc)]

    def lhs_448(ref, r0, nr):
        rs = slice(r0 // 2, (r0 + nr) // 2)
        return jnp.concatenate([_as_bf16(ref[0, rs, :]), _as_bf16(ref[1, rs, :]), _as_bf16(ref[2, rs, :]),
                                _as_bf16(ref[3, rs, :])[:, 0:64]], axis=1)

    def qkv_store(j, sec, res):
        if sec == 0:
            q_s[j] = res
        else:
            dst = k_s if sec == 1 else v_s
            for d in range(DH):
                dst[j, 8 * d:8 * d + 8, :] = _pack(res[16 * d:16 * d + 8], res[16 * d + 8:16 * d + 16])

    def qkv(j, sec):
        if QONE:
            if sec == 0:
                wt = lhs_448(wt_s, 0, 3 * D)
                res = jnp.dot(wt, _as_bf16(xn_s[:, lt(j)]), preferred_element_type=f32)
                for s3 in range(3):
                    qkv_store(j, s3, res[s3 * D:(s3 + 1) * D])
                qkv.res = res
            return qkv.res[sec * D:sec * D + 8]
        wt = lhs_448(wt_s, sec * D, D)
        res = jnp.dot(wt, _as_bf16(xn_s[:, lt(j)]), preferred_element_type=f32)
        qkv_store(j, sec, res)
        return res[0:8]

    def shifted(cur, prev, w):
        if w == 0:
            return cur
        sh = DIL * w
        return pltpu.roll(jnp.where(lane >= 128 - sh, prev, cur), sh, 1)

    def attention(j):
        jp = max(j - 1, 0)
        acc = [[None, None] for _ in range(W)]
        for d in range(DH):
            q = [q_s[j, 16 * d + 8 * g:16 * d + 8 * g + 8, :] for g in range(2)]
            k = k_s[j, 8 * d:8 * d + 8, :]
            kp = k_s[jp, 8 * d:8 * d + 8, :]
            for w in range(W):
                ks = shifted(k, kp, w)
                for g in range(2):
                    p = q[g] * _unpack(ks, g)
                    acc[w][g] = p if acc[w][g] is None else acc[w][g] + p
        scale = DH ** -0.5
        prob = [[None, None] for _ in range(W)]
        for g in range(2):
            if SMX:
                lg = [acc[w][g] for w in range(W)]
                if j == 0:
                    lg = [lg[w] if w == 0 else jnp.where(lane >= DIL * w, lg[w], -1e9 / scale) for w in range(W)]
                m = lg[0]
                for w in range(1, W):
                    m = jnp.maximum(m, lg[w])
                e = [jnp.exp2((t - m) * (scale * 1.4426950408889634)) for t in lg]
            else:
                lg = [acc[w][g] * scale for w in range(W)]
                if j == 0:
                    lg = [lg[w] if w == 0 else jnp.where(lane >= DIL * w, lg[w], -1e9) for w in range(W)]
                m = lg[0]
                for w in range(1, W):
                    m = jnp.maximum(m, lg[w])
                e = [jnp.exp(t - m) for t in lg]
            inv = 1.0 / _tree_sum(e)
            for w in range(W):
                prob[w][g] = e[w] * inv
        for d in range(DH):
            v = v_s[j, 8 * d:8 * d + 8, :]
            vp = v_s[jp, 8 * d:8 * d + 8, :]
            o = [None, None]
            for w in range(W):
                vs = shifted(v, vp, w)
                for g in range(2):
                    p = prob[w][g] * _unpack(vs, g)
                    o[g] = p if o[g] is None else o[g] + p
            o_s[j, 8 * d:8 * d + 8, :] = _pack(o[0], o[1])

    def oproj(j):
        wot = lhs_448(wot_s, 0, D)
        a = jnp.dot(wot, _as_bf16(o_s[j]), preferred_element_type=f32)
        b2 = b2_s[pl.ds(128 * j, 128)].astype(f32).reshape(1, 128)
        r_s[j] = a + _as_bf16(x_s[:, lt(j)]).astype(f32) + b2

    def mixer_up(t0, nt, c0, nc):
        hb = _as_bf16(h_s[:, lt(t0, nt)])
        wb = _as_bf16(w1_s[64 * t0:64 * (t0 + nt), lt(c0, nc)])
        upd = jnp.dot(hb, wb, preferred_element_type=f32)
        if t0 == 0:
            u_s[:, lt(c0, nc)] = upd
        elif t0 + nt < NT:
            u_s[:, lt(c0, nc)] = u_s[:, lt(c0, nc)] + upd
        else:
            b1 = b1_s[pl.ds(128 * c0, 128 * nc)].astype(f32).reshape(1, 128 * nc)
            t = u_s[:, lt(c0, nc)] + upd + b1
            ub_s[:, lt(c0, nc)] = pltpu.bitcast(jax.nn.gelu(t, approximate=True).astype(bf16), u32)
        return upd[0:8, 0:128]

    def mixer_down(j0, nj):
        ub = _as_bf16(ub_s[...])
        if isinstance(j0, int):
            cols = lambda t, n: lt(j0 + t, n)
        else:
            cols = lambda t, n: pl.ds(pl.multiple_of((j0 + t) * 128, 128), 128 * n)
        y = jnp.dot(ub, _as_bf16(w2_s[:, cols(0, nj)]), preferred_element_type=f32)
        for t in range(nj):
            out_s[:, cols(t, 1)] = pltpu.bitcast((y[:, lt(t)] + r_s[j0 + t]).astype(bf16), u32)

    def tiles(b):
        return range(KB * b, KB * b + KB)

    tok = None
    n_first = 2 if KSPLIT else KB
    for j in range(n_first):
        cp_x[j].wait(tok)
        tok = layer_norms(j)
    ln_at = {}
    for j, p in LN_A_AT.items():
        ln_at.setdefault(p, []).append(j)
    for p, piece in enumerate(start):
        if p in cp_start:
            cp_start[p].wait(tok)
        tok = mixer_up(*piece)
        if KSPLIT and p in LN23_AT:
            jx = 2 + LN23_AT.index(p)
            cp_x[jx].wait(tok)
            layer_norms(jx, tok)
        if p == min(LN_A_AT[j] for j in range(KB, 2 * KB)):
            cp_x1.wait(tok)
        if p == min(LN_A_AT[j] for j in range(2 * KB, 3 * KB)):
            cp_x2.wait(tok)
        for i in range(4):
            if PREP_AT[i] == p:
                cp_wqkv[i].wait(tok)
                prep_wqkv(i, tok)
        for j in ln_at.get(p, ()):
            layer_norms(j, tok)

    def out_copy(j0, n, sem):
        if isinstance(j0, int):
            sl = lt(j0, n)
        else:
            sl = pl.ds(pl.multiple_of(j0 * 128, 128), 128 * n)
        return pltpu.make_async_copy(out_s.at[:, sl], out_hbm.at[:, sl], sems.at[sem])

    for b in range(NB):
        kb, hf = b // 2, b % 2
        for t, j in enumerate(tiles(b)):
            for sec in range(3):
                tok = qkv(j, sec)
                if b == 0:
                    for i in range(4):
                        if PREP_WO_AT[i] == 3 * t + sec:
                            if i == 0:
                                cp_wo.wait(tok)
                                cp_b2.wait(tok)
                            prep_wo(i, tok)
                if t == KB - 1 and sec == 1:
                    cp_w1[kb, hf].wait(tok)
                    if b == 0:
                        cp_x3.wait(tok)
                    if b == 2:
                        cp_b1.wait(tok)
                    if b == NB - 1:
                        for c in cp_w2:
                            c.wait(tok)
            attention(j)
        for i in range(7):
            tok = mixer_up(KB * (2 + kb), KB, 7 * hf + i, 1)
            for j, at in LN_B_AT.items():
                if at == (b, i):
                    layer_norms(j, tok)
        for j in tiles(b):
            oproj(j)
    mixer_down(0, 2)
    s0 = sem_i[0]
    out_copy(0, 2, s0).start()

    def body(i, carry):
        j0 = 2 + 2 * LOOP_P * i
        for p in range(LOOP_P):
            mixer_down(j0 + 2 * p, 2)
        out_copy(j0, 2 * LOOP_P, s0 + 1 + i).start()
        return carry

    jax.lax.fori_loop(0, LOOP_N, body, 0)
    jt = 2 + 2 * LOOP_P * LOOP_N
    for j0 in range(jt, NT, 2):
        mixer_down(j0, 2)
    out_copy(jt, NT - jt, s0 + 1 + LOOP_N).start()
    out_copy(0, 2, s0).wait()
    for i in range(LOOP_N):
        out_copy(2 + 2 * LOOP_P * i, 2 * LOOP_P, s0 + 1 + i).wait()
    out_copy(jt, NT - jt, s0 + 1 + LOOP_N).wait()


@jax.jit
def pallas_parallel_sum__sliding_local_dilated__mixer_token_mlp__prompt_kernel(
    A_x, A_wqkv, A_wo, B_x, B_w1, B_b1, B_w2, B_b2,
):
    del B_x
    xT = A_x.reshape(S, D).T
    any_spec = pl.BlockSpec(memory_space=pl.ANY)
    scratch = [
        pltpu.VMEM((D // 2, S), u32),
        pltpu.VMEM((D // 2, 3 * D), u32),
        pltpu.VMEM((D // 2, D), u32),
        pltpu.VMEM((S // 2, F), u32),
        pltpu.VMEM((F // 2, S), u32),
        pltpu.VMEM((F,), bf16),
        pltpu.VMEM((S,), bf16),
        pltpu.VMEM((4, 24 * 57, 128), f32),
        pltpu.VMEM((4, D // 2, 128), u32),
        pltpu.VMEM((4, 3 * D // 2, 128), u32),
        pltpu.VMEM((4, D // 2, 128), u32),
        pltpu.VMEM((D // 2, S), u32),
        pltpu.VMEM((D // 2, S), u32),
        pltpu.VMEM((NT, D, 128), f32),
        pltpu.VMEM((NT, D // 2, 128), u32),
        pltpu.VMEM((NT, D // 2, 128), u32),
        pltpu.VMEM((NT, D, 128), u32),
        pltpu.VMEM((NT, D, 128), f32),
        pltpu.VMEM((D, F), f32),
        pltpu.VMEM((D // 2, F), u32),
        pltpu.VMEM((D // 2, S), u32),
        pltpu.SemaphoreType.DMA((N_SEMS,)),
    ]
    scratch[16] = pltpu.VMEM((NT, D // 2, 128), u32)
    outT = pl.pallas_call(
        _kernel,
        out_shape=jax.ShapeDtypeStruct((D, S), bf16),
        in_specs=[any_spec] * 7,
        out_specs=any_spec,
        scratch_shapes=scratch,
        compiler_params=pltpu.CompilerParams(vmem_limit_bytes=100 * 1024 * 1024, flags=FLAGS, disable_bounds_checks=True, disable_semaphore_checks=True),
        name="fused_kernel",
    )(xT, A_wqkv, A_wo, B_w1, B_b1, B_w2, B_b2)
    return outT.T.reshape(1, S, D)
```

```python
import jax
import jax.numpy as jnp
import numpy as np
import jax.experimental.pallas as pl
import jax.experimental.pallas.tpu as pltpu

S, D, H, DH, F = 2048, 448, 16, 28, 1792
W, DIL = 8, 2
NT = S // 128
NF = F // 128
EPS = 1e-5
f32, bf16, u32, i32 = jnp.float32, jnp.bfloat16, jnp.uint32, jnp.int32


def _unpack(x, i):
    return pltpu.unpack_elementwise(x, index=i, packed_dtype=bf16, unpacked_dtype=f32)


def _unpack2(x, i):
    if i == 0:
        return jax.lax.bitcast_convert_type(x << 16, f32)
    return jax.lax.bitcast_convert_type(x & jnp.uint32(0xFFFF0000), f32)


def _pack(a, b):
    return pltpu.pack_elementwise([a, b], packed_dtype=bf16)


def _as_bf16(x_u32):
    return pltpu.bitcast(x_u32, bf16)


def _tree_sum(xs):
    xs = list(xs)
    while len(xs) > 1:
        nxt = [xs[i] + xs[i + 1] for i in range(0, len(xs) - 1, 2)]
        if len(xs) % 2:
            nxt.append(xs[-1])
        xs = nxt
    return xs[0]


def _bcast_rows_sum(p):
    t = jnp.sum(p, axis=0, keepdims=True)
    return jnp.broadcast_to(t, (8, 128))


def _never(tok):
    return tok * tok < -1.0


def _zero_after(tok):
    return jnp.where(_never(tok), 1.0, 0.0).astype(f32)


KB = 4
NB = NT // KB
LOOP_N, LOOP_P = (2, 3)
QONE = 1
SMX = 1
DMA_AFTER_C = {0: ('q',), 2: ('q',), 3: ('q',), 5: ('q',), 6: ('x2', 'wo')}
X23_AFTER = (5, 6)
LN23_AT = (4, 5)
NACC = 2
PVDEP = 1
X1T_AFTER = 1
LN1_AT = 1
LN_Q_AT = {9: 0, 10: 1, 11: 2}
PREP_WO_F = (2, 3, 4, 5)
X2_WAIT = 27
KSPLIT = 2
LN_A_AT = {4: 8, 5: 10, 6: 11, 7: 12, 8: 27}
LN_B_AT = {12: (1, 3), 13: (1, 4), 14: (1, 5), 15: (1, 6)}
PREP_AT = (14, 18, 21, 25)
PREP_WO_AT = (0, 1, 2, 3)
FLAGS = {"XLA_TPU_RESCHEDULE_DMA_DONES": True, "XLA_TPU_EVENLY_DISTRIBUTE_CRITICAL_NODES": True}
N_SEMS = 64


def _kernel(x_hbm, wqkv_hbm, wo_hbm, w1_hbm, b1_hbm, w2_hbm, b2_hbm, out_hbm,
            x_s, wqkv_s, wo_s, w1_s, w2_s, b1_s, b2_s,
            wt_f, wo_f, wt_s, wot_s,
            xn_s, h_s, q_s, k_s, v_s, o_s, r_s, u_s, ub_s, out_s, sems):
    x_hbm, wqkv_hbm, wo_hbm, w1_hbm, w2_hbm, out_hbm = (
        r.bitcast(u32) for r in (x_hbm, wqkv_hbm, wo_hbm, w1_hbm, w2_hbm, out_hbm))
    sem_i = [0]

    class Dma:
        def __init__(self, src, dst):
            self.src, self.dst, self.i = src, dst, sem_i[0]
            sem_i[0] += 1
            pltpu.make_async_copy(src, dst, sems.at[self.i]).start()

        def wait(self, tok=None):
            idx = self.i
            if tok is not None:
                idx = idx + jnp.where(_never(tok), 1, 0).astype(i32)[0, 0]
            pltpu.make_async_copy(self.src, self.dst, sems.at[idx]).wait()

    def lt(j, n=1):
        return slice(128 * j, 128 * (j + n))

    def x_dma(j, n):
        return Dma(x_hbm.at[:, lt(j, n)], x_s.at[:, lt(j, n)])

    def w1_dma(t0, nt, c0=0, n=NF):
        rows = pl.ds(64 * t0, 64 * nt)
        return Dma(w1_hbm.at[rows, lt(c0, n)], w1_s.at[rows, lt(c0, n)])

    def wqkv_dma(c):
        rows = pl.ds(64 * c, min(64, D // 2 - 64 * c))
        return Dma(wqkv_hbm.at[rows], wqkv_s.at[rows])

    if KSPLIT == 2:
        start = [[(0, 1, 0, 4)], [(0, 1, 4, 4)], [(0, 1, 8, 4)], [(0, 1, 12, 2), (1, 1, 0, 2)],
                 [(1, 1, 2, 4)], [(1, 1, 6, 4)], [(1, 1, 10, 4)]]
        start += [[(2, 2, 2 * i, 2)] for i in range(NF // 2)]
    elif KSPLIT == 1:
        start = [[(0, 2, 2 * i, 2)] for i in range(NF // 2)] + [[(2, 2, 2 * i, 2)] for i in range(NF // 2)]
    else:
        start = [[(0, 4, c, 1)] for c in range(NF)]
    start += [[(4, 4, c, 1)] for c in range(NF)]

    cp_x = {}
    cp_start = {}
    cp_wqkv = []
    if KSPLIT:
        cp_x[0] = x_dma(0, 1)
        if KSPLIT == 1:
            cp_x[1] = x_dma(1, 1)
        for i in range(NF // 2):
            cp_start[i] = [w1_dma(*dot) for dot in start[i]]
            if KSPLIT == 2 and i == X1T_AFTER:
                cp_x[1] = x_dma(1, 1)
            if i in X23_AFTER:
                jx = 2 + X23_AFTER.index(i)
                cp_x[jx] = x_dma(jx, 1)
        for i in range(NF // 2):
            cp_start[NF // 2 + i] = [w1_dma(2, 2, 2 * i, 2)]
            if i == 1:
                cp_x1 = x_dma(KB, KB)
    else:
        for j in range(KB):
            cp_x[j] = x_dma(j, 1)
        for i in range(NF // 2):
            cp_start[2 * i] = [w1_dma(0, 4, 2 * i, 2)]
            if i == 2:
                cp_x1 = x_dma(KB, KB)
    for i in range(NF // 2):
        cp_start[NF + 2 * i] = [w1_dma(4, 4, 2 * i, 2)]
        for extra in DMA_AFTER_C.get(i, ()):
            if extra == "x2":
                cp_x2 = x_dma(2 * KB, KB)
            elif extra == "wo":
                cp_wo = Dma(wo_hbm, wo_s)
                cp_b2 = Dma(b2_hbm, b2_s)
            else:
                cp_wqkv.append(wqkv_dma(len(cp_wqkv)))
    cp_x3 = x_dma(3 * KB, KB)
    cp_b1 = Dma(b1_hbm, b1_s)
    cp_w1 = {(b, hf): w1_dma(KB * (2 + b), KB, 7 * hf, 7) for b in range(2) for hf in range(2)}
    cp_w2 = [Dma(w2_hbm.at[:, lt(4 * b, 4)], w2_s.at[:, lt(4 * b, 4)]) for b in range(4)]

    lane = jax.lax.broadcasted_iota(jnp.int32, (8, 128), 1)

    def layer_norms(j, dep=None):
        n16 = D // 16
        k0 = jnp.broadcast_to(_unpack(x_s[0:8, lt(j)], 0)[0:1, :], (8, 128))
        if dep is not None:
            k0 = k0 + _zero_after(dep)
        s1, s2 = [None, None], [None, None]
        for i in range(n16):
            p = x_s[8 * i:8 * i + 8, lt(j)]
            for t in range(2):
                c = _unpack(p, t) - k0
                a = t % NACC
                s1[a] = c if s1[a] is None else s1[a] + c
                s2[a] = c * c if s2[a] is None else s2[a] + c * c
        m1 = _bcast_rows_sum(sum(s1[1:NACC], s1[0])) * (1.0 / D)
        m2 = _bcast_rows_sum(sum(s2[1:NACC], s2[0])) * (1.0 / D)
        mean = k0 + m1
        rstd = jax.lax.rsqrt(jnp.maximum(m2 - m1 * m1, 0.0) + EPS)
        t1, t2 = [None, None], [None, None]
        for i in range(n16):
            p = x_s[8 * i:8 * i + 8, lt(j)]
            xs = []
            for t in range(2):
                xn = (_unpack2(p, t) - mean) * rstd
                xs.append(xn)
                a = t % NACC
                t1[a] = xn if t1[a] is None else t1[a] + xn
                t2[a] = xn * xn if t2[a] is None else t2[a] + xn * xn
            xn_s[8 * i:8 * i + 8, lt(j)] = _pack(xs[0], xs[1])
        mean2 = _bcast_rows_sum(sum(t1[1:NACC], t1[0])) * (1.0 / D)
        e2 = _bcast_rows_sum(sum(t2[1:NACC], t2[0])) * (1.0 / D)
        rstd2 = jax.lax.rsqrt(jnp.maximum(e2 - mean2 * mean2, 0.0) + EPS)
        for i in range(n16):
            p = xn_s[8 * i:8 * i + 8, lt(j)]
            h_s[8 * i:8 * i + 8, lt(j)] = _pack((_unpack(p, 0) - mean2) * rstd2, (_unpack(p, 1) - mean2) * rstd2)
        return rstd2

    ST = 57

    def prep_wqkv(c, dep):
        rows = min(128, D - 128 * c)
        wp = wqkv_s[64 * c:64 * c + rows // 2, :]
        wp = jnp.where(jnp.tile(_never(dep), (rows // 16, 11))[:, :3 * D], jnp.uint32(0), wp)
        w = _as_bf16(wp).astype(f32)
        if rows < 128:
            w = jnp.concatenate([w, jnp.zeros((128 - rows, 3 * D), f32)], axis=0)
        wt = w.T
        for v in range(3 * D // 8):
            wt_f[c, pl.ds(8 * v + (8 * v) // 56, 8), :] = wt[8 * v:8 * v + 8]
        for sec in range(3):
            for d in range(DH):
                ev, od = (wt_f[c, pl.ds(sec * 8 * ST + DH * g + d, 8, stride=ST), :] for g in range(2))
                wt_s[c, sec * (D // 2) + 8 * d:sec * (D // 2) + 8 * d + 8, :] = _pack(ev, od)

    def prep_wo(c, dep):
        cols = min(128, D - 128 * c)
        wp = wo_s[:, 128 * c:128 * c + cols]
        wp = jnp.where(jnp.tile(_never(dep), (D // 16, 1))[:, :cols], jnp.uint32(0), wp)
        if cols < 128:
            wp = jnp.concatenate([wp, jnp.zeros((D // 2, 128 - cols), u32)], axis=1)
        wo_f[c] = wp
        parts = []
        for dp in range(DH // 2):
            gath = [wo_f[c, pl.ds(14 * 8 * g + dp, 8, stride=14), :] for g in range(2)]
            for e in range(2):
                parts.append(_pack(_unpack(gath[0], e), _unpack(gath[1], e)))
        wpk = _as_bf16(jnp.concatenate(parts, axis=0))
        wpk = jnp.concatenate([wpk, jnp.zeros((512 - D, 128), bf16)], axis=0)
        wpt = pltpu.bitcast(wpk.T, u32)
        rows = min(128, D - 128 * c) // 2
        for cc in range(4):
            wot_s[cc, 64 * c:64 * c + rows, :] = wpt[:rows, lt(cc)]

    def lhs_448(ref, r0, nr):
        rs = slice(r0 // 2, (r0 + nr) // 2)
        return jnp.concatenate([_as_bf16(ref[0, rs, :]), _as_bf16(ref[1, rs, :]), _as_bf16(ref[2, rs, :]),
                                _as_bf16(ref[3, rs, :])[:, 0:64]], axis=1)

    def qkv_store(j, sec, res):
        if sec == 0:
            q_s[j] = res
        else:
            dst = k_s if sec == 1 else v_s
            for d in range(DH):
                dst[j, 8 * d:8 * d + 8, :] = _pack(res[16 * d:16 * d + 8], res[16 * d + 8:16 * d + 16])

    def qkv(j, sec):
        if QONE:
            if sec == 0:
                wt = lhs_448(wt_s, 0, 3 * D)
                res = jnp.dot(wt, _as_bf16(xn_s[:, lt(j)]), preferred_element_type=f32)
                for s3 in range(3):
                    qkv_store(j, s3, res[s3 * D:(s3 + 1) * D])
                qkv.res = res
            return qkv.res[sec * D:sec * D + 8]
        wt = lhs_448(wt_s, sec * D, D)
        res = jnp.dot(wt, _as_bf16(xn_s[:, lt(j)]), preferred_element_type=f32)
        qkv_store(j, sec, res)
        return res[0:8]

    def shifted(cur, prev, w):
        if w == 0:
            return cur
        sh = DIL * w
        return pltpu.roll(jnp.where(lane >= 128 - sh, prev, cur), sh, 1)

    def attention(j):
        jp = max(j - 1, 0)
        acc = [[None, None] for _ in range(W)]
        for d in range(DH):
            q = [q_s[j, 16 * d + 8 * g:16 * d + 8 * g + 8, :] for g in range(2)]
            k = k_s[j, 8 * d:8 * d + 8, :]
            kp = k_s[jp, 8 * d:8 * d + 8, :]
            for w in range(W):
                ks = shifted(k, kp, w)
                for g in range(2):
                    p = q[g] * _unpack(ks, g)
                    acc[w][g] = p if acc[w][g] is None else acc[w][g] + p
        scale = DH ** -0.5
        prob = [[None, None] for _ in range(W)]
        for g in range(2):
            if SMX:
                lg = [acc[w][g] for w in range(W)]
                if j == 0:
                    lg = [lg[w] if w == 0 else jnp.where(lane >= DIL * w, lg[w], -1e9 / scale) for w in range(W)]
                m = lg[0]
                for w in range(1, W):
                    m = jnp.maximum(m, lg[w])
                e = [jnp.exp2((t - m) * (scale * 1.4426950408889634)) for t in lg]
            else:
                lg = [acc[w][g] * scale for w in range(W)]
                if j == 0:
                    lg = [lg[w] if w == 0 else jnp.where(lane >= DIL * w, lg[w], -1e9) for w in range(W)]
                m = lg[0]
                for w in range(1, W):
                    m = jnp.maximum(m, lg[w])
                e = [jnp.exp(t - m) for t in lg]
            esum = _tree_sum(e)
            e_tok = esum
            inv = 1.0 / esum
            for w in range(W):
                prob[w][g] = e[w] * inv
        pv_mask = _never(e_tok)
        for d in range(DH):
            v = v_s[j, 8 * d:8 * d + 8, :]
            vp = v_s[jp, 8 * d:8 * d + 8, :]
            if PVDEP == 1 or (PVDEP == 2 and d < 4):
                v = jnp.where(pv_mask, jnp.uint32(0), v)
            o = [None, None]
            for w in range(W):
                vs = shifted(v, vp, w)
                for g in range(2):
                    p = prob[w][g] * _unpack(vs, g)
                    o[g] = p if o[g] is None else o[g] + p
            o_s[j, 8 * d:8 * d + 8, :] = _pack(o[0], o[1])

    def oproj(j):
        wot = lhs_448(wot_s, 0, D)
        a = jnp.dot(wot, _as_bf16(o_s[j]), preferred_element_type=f32)
        b2 = b2_s[pl.ds(128 * j, 128)].astype(f32).reshape(1, 128)
        r_s[j] = a + _as_bf16(x_s[:, lt(j)]).astype(f32) + b2

    def mixer_up(t0, nt, c0, nc):
        hb = _as_bf16(h_s[:, lt(t0, nt)])
        wb = _as_bf16(w1_s[64 * t0:64 * (t0 + nt), lt(c0, nc)])
        upd = jnp.dot(hb, wb, preferred_element_type=f32)
        if t0 == 0:
            u_s[:, lt(c0, nc)] = upd
        elif t0 + nt < NT:
            u_s[:, lt(c0, nc)] = u_s[:, lt(c0, nc)] + upd
        else:
            b1 = b1_s[pl.ds(128 * c0, 128 * nc)].astype(f32).reshape(1, 128 * nc)
            t = u_s[:, lt(c0, nc)] + upd + b1
            ub_s[:, lt(c0, nc)] = pltpu.bitcast(jax.nn.gelu(t, approximate=True).astype(bf16), u32)
        return upd[0:8, 0:128]

    def mixer_down(j0, nj):
        ub = _as_bf16(ub_s[...])
        if isinstance(j0, int):
            cols = lambda t, n: lt(j0 + t, n)
        else:
            cols = lambda t, n: pl.ds(pl.multiple_of((j0 + t) * 128, 128), 128 * n)
        y = jnp.dot(ub, _as_bf16(w2_s[:, cols(0, nj)]), preferred_element_type=f32)
        for t in range(nj):
            out_s[:, cols(t, 1)] = pltpu.bitcast((y[:, lt(t)] + r_s[j0 + t]).astype(bf16), u32)

    def tiles(b):
        return range(KB * b, KB * b + KB)

    tok = None
    n_first = {0: KB, 1: 2, 2: 1}[KSPLIT]
    for j in range(n_first):
        cp_x[j].wait(tok)
        tok = layer_norms(j)
    ln_at = {}
    for j, p in LN_A_AT.items():
        ln_at.setdefault(p, []).append(j)
    for p, piece in enumerate(start):
        for c in cp_start.get(p, ()):
            c.wait(tok)
        toks = [mixer_up(*dot) for dot in piece]
        tok = toks[0]
        if KSPLIT == 2 and p == LN1_AT:
            cp_x[1].wait(tok)
            layer_norms(1, tok)
        if KSPLIT and p in LN23_AT:
            jx = 2 + LN23_AT.index(p)
            cp_x[jx].wait(tok)
            layer_norms(jx, tok)
        if p == min(LN_A_AT[j] for j in range(KB, 2 * KB)):
            cp_x1.wait(tok)
        if p == (X2_WAIT if X2_WAIT >= 0 else min(LN_A_AT[j] for j in range(2 * KB, 3 * KB))):
            cp_x2.wait(tok)
        for i in range(4):
            if PREP_AT[i] == p:
                cp_wqkv[i].wait(tok)
                prep_wqkv(i, tok)
        for j in ln_at.get(p, ()):
            layer_norms(j, tok)

    def out_copy(j0, n, sem):
        if isinstance(j0, int):
            sl = lt(j0, n)
        else:
            sl = pl.ds(pl.multiple_of(j0 * 128, 128), 128 * n)
        return pltpu.make_async_copy(out_s.at[:, sl], out_hbm.at[:, sl], sems.at[sem])

    for b in range(NB):
        kb, hf = b // 2, b % 2
        for t, j in enumerate(tiles(b)):
            for sec in range(3):
                tok = qkv(j, sec)
                if b == 0:
                    for jj, at in LN_Q_AT.items():
                        if at == 3 * t + sec:
                            layer_norms(jj, tok)
                    for i in range(4):
                        if PREP_WO_F is None and PREP_WO_AT[i] == 3 * t + sec:
                            if i == 0:
                                cp_wo.wait(tok)
                                cp_b2.wait(tok)
                            prep_wo(i, tok)
                if t == KB - 1 and sec == 1:
                    cp_w1[kb, hf].wait(tok)
                    if b == 0:
                        cp_x3.wait(tok)
                    if b == 2:
                        cp_b1.wait(tok)
                    if b == NB - 1:
                        for c in cp_w2:
                            c.wait(tok)
            attention(j)
        for i in range(7):
            tok = mixer_up(KB * (2 + kb), KB, 7 * hf + i, 1)
            for j, at in LN_B_AT.items():
                if at == (b, i):
                    layer_norms(j, tok)
            if b == 0 and PREP_WO_F is not None:
                for ii in range(4):
                    if PREP_WO_F[ii] == i:
                        if ii == 0:
                            cp_wo.wait(tok)
                            cp_b2.wait(tok)
                        prep_wo(ii, tok)
        for j in tiles(b):
            oproj(j)
    mixer_down(0, 2)
    s0 = sem_i[0]
    out_copy(0, 2, s0).start()

    def body(i, carry):
        j0 = 2 + 2 * LOOP_P * i
        for p in range(LOOP_P):
            mixer_down(j0 + 2 * p, 2)
        out_copy(j0, 2 * LOOP_P, s0 + 1 + i).start()
        return carry

    jax.lax.fori_loop(0, LOOP_N, body, 0)
    jt = 2 + 2 * LOOP_P * LOOP_N
    for j0 in range(jt, NT, 2):
        mixer_down(j0, 2)
    out_copy(jt, NT - jt, s0 + 1 + LOOP_N).start()
    out_copy(0, 2, s0).wait()
    for i in range(LOOP_N):
        out_copy(2 + 2 * LOOP_P * i, 2 * LOOP_P, s0 + 1 + i).wait()
    out_copy(jt, NT - jt, s0 + 1 + LOOP_N).wait()


@jax.jit
def pallas_parallel_sum__sliding_local_dilated__mixer_token_mlp__prompt_kernel(
    A_x, A_wqkv, A_wo, B_x, B_w1, B_b1, B_w2, B_b2,
):
    del B_x
    xT = A_x.reshape(S, D).T
    any_spec = pl.BlockSpec(memory_space=pl.ANY)
    scratch = [
        pltpu.VMEM((D // 2, S), u32),
        pltpu.VMEM((D // 2, 3 * D), u32),
        pltpu.VMEM((D // 2, D), u32),
        pltpu.VMEM((S // 2, F), u32),
        pltpu.VMEM((F // 2, S), u32),
        pltpu.VMEM((F,), bf16),
        pltpu.VMEM((S,), bf16),
        pltpu.VMEM((4, 24 * 57, 128), f32),
        pltpu.VMEM((4, D // 2, 128), u32),
        pltpu.VMEM((4, 3 * D // 2, 128), u32),
        pltpu.VMEM((4, D // 2, 128), u32),
        pltpu.VMEM((D // 2, S), u32),
        pltpu.VMEM((D // 2, S), u32),
        pltpu.VMEM((NT, D, 128), f32),
        pltpu.VMEM((NT, D // 2, 128), u32),
        pltpu.VMEM((NT, D // 2, 128), u32),
        pltpu.VMEM((NT, D, 128), u32),
        pltpu.VMEM((NT, D, 128), f32),
        pltpu.VMEM((D, F), f32),
        pltpu.VMEM((D // 2, F), u32),
        pltpu.VMEM((D // 2, S), u32),
        pltpu.SemaphoreType.DMA((N_SEMS,)),
    ]
    scratch[16] = pltpu.VMEM((NT, D // 2, 128), u32)
    outT = pl.pallas_call(
        _kernel,
        out_shape=jax.ShapeDtypeStruct((D, S), bf16),
        in_specs=[any_spec] * 7,
        out_specs=any_spec,
        scratch_shapes=scratch,
        compiler_params=pltpu.CompilerParams(vmem_limit_bytes=100 * 1024 * 1024, flags=FLAGS, disable_bounds_checks=True, disable_semaphore_checks=True),
        name="fused_kernel",
    )(xT, A_wqkv, A_wo, B_w1, B_b1, B_w2, B_b2)
    return outT.T.reshape(1, S, D)
```

```python
import jax
import jax.numpy as jnp
import jax.experimental.pallas as pl
import jax.experimental.pallas.tpu as pltpu

S, D, H, DH, F = 2048, 448, 16, 28, 1792
W, DIL = 8, 2
NT = S // 128
NF = F // 128
KB = 4
NB = NT // KB
EPS = 1e-5
ST = 57
f32, bf16, u32, i32 = jnp.float32, jnp.bfloat16, jnp.uint32, jnp.int32

START = ([[(0, 1, 0, 4)], [(0, 1, 4, 4)], [(0, 1, 8, 4)], [(0, 1, 12, 2), (1, 1, 0, 2)],
          [(1, 1, 2, 4)], [(1, 1, 6, 4)], [(1, 1, 10, 4)]]
         + [[(2, 2, 2 * i, 2)] for i in range(NF // 2)]
         + [[(4, 4, c, 1)] for c in range(NF)])
LN_IN_START = {1: 1, 2: 4, 3: 5, 4: 8, 5: 10, 6: 11, 7: 12, 8: 27}
LN_IN_QKV = {9: 0, 10: 1, 11: 2}
LN_IN_FILL = {12: 3, 13: 4, 14: 5, 15: 6}
WQKV_PREP_AT = (14, 18, 21, 25)
WO_PREP_AT = (2, 3, 4, 5)
LOOP_N, LOOP_P = 2, 3
N_SEMS = 48


def _unpack(x, i):
    return pltpu.unpack_elementwise(x, index=i, packed_dtype=bf16, unpacked_dtype=f32)


def _unpack_bits(x, i):
    if i == 0:
        return jax.lax.bitcast_convert_type(x << 16, f32)
    return jax.lax.bitcast_convert_type(x & jnp.uint32(0xFFFF0000), f32)


def _pack(lo, hi):
    return pltpu.pack_elementwise([lo, hi], packed_dtype=bf16)


def _as_bf16(x_u32):
    return pltpu.bitcast(x_u32, bf16)


def _tree_sum(xs):
    xs = list(xs)
    while len(xs) > 1:
        nxt = [xs[i] + xs[i + 1] for i in range(0, len(xs) - 1, 2)]
        if len(xs) % 2:
            nxt.append(xs[-1])
        xs = nxt
    return xs[0]


def _col_sum(p):
    return jnp.broadcast_to(jnp.sum(p, axis=0, keepdims=True), (8, 128))


def _never(tok):
    return tok * tok < -1.0


def _zero_after(tok):
    return jnp.where(_never(tok), 1.0, 0.0).astype(f32)


def _kernel(x_hbm, wqkv_hbm, wo_hbm, w1_hbm, b1_hbm, w2_hbm, b2_hbm, out_hbm,
            x_s, wqkv_s, wo_s, w1_s, w2_s, b1_s, b2_s,
            wt_f, wo_f, wt_s, wot_s,
            xn_s, h_s, q_s, k_s, v_s, o_s, r_s, u_s, ub_s, out_s, sems):
    x_hbm, wqkv_hbm, wo_hbm, w1_hbm, w2_hbm, out_hbm = (
        r.bitcast(u32) for r in (x_hbm, wqkv_hbm, wo_hbm, w1_hbm, w2_hbm, out_hbm))

    def lt(j, n=1):
        return slice(128 * j, 128 * (j + n))

    n_sem = [0]

    class Dma:
        def __init__(self, src, dst):
            self.src, self.dst, self.sem = src, dst, n_sem[0]
            n_sem[0] += 1
            pltpu.make_async_copy(src, dst, sems.at[self.sem]).start()

        def wait(self, tok=None):
            sem = self.sem
            if tok is not None:
                sem = sem + jnp.where(_never(tok), 1, 0).astype(i32)[0, 0]
            pltpu.make_async_copy(self.src, self.dst, sems.at[sem]).wait()

    def x_dma(j, n):
        return Dma(x_hbm.at[:, lt(j, n)], x_s.at[:, lt(j, n)])

    def w1_dma(t0, nt, c0, nc):
        rows = pl.ds(64 * t0, 64 * nt)
        return Dma(w1_hbm.at[rows, lt(c0, nc)], w1_s.at[rows, lt(c0, nc)])

    def wqkv_dma(c):
        rows = pl.ds(64 * c, min(64, D // 2 - 64 * c))
        return Dma(wqkv_hbm.at[rows], wqkv_s.at[rows])

    cp_x = {0: x_dma(0, 1)}
    cp_start = {}
    for p in range(7):
        cp_start[p] = [w1_dma(*dot) for dot in START[p]]
        if p in (1, 5, 6):
            j = {1: 1, 5: 2, 6: 3}[p]
            cp_x[j] = x_dma(j, 1)
    for i in range(7):
        cp_start[7 + i] = [w1_dma(2, 2, 2 * i, 2)]
        if i == 1:
            cp_x[4] = x_dma(4, 4)
    cp_wqkv = []
    for i in range(7):
        cp_start[14 + 2 * i] = [w1_dma(4, 4, 2 * i, 2)]
        if i in (0, 2, 3, 5):
            cp_wqkv.append(wqkv_dma(len(cp_wqkv)))
    cp_x[8] = x_dma(8, 4)
    cp_wo = Dma(wo_hbm, wo_s)
    cp_b2 = Dma(b2_hbm, b2_s)
    cp_x[12] = x_dma(12, 4)
    cp_b1 = Dma(b1_hbm, b1_s)
    cp_w1 = [w1_dma(KB * (2 + b // 2), KB, 7 * (b % 2), 7) for b in range(NB)]
    cp_w2 = [Dma(w2_hbm.at[:, lt(4 * i, 4)], w2_s.at[:, lt(4 * i, 4)]) for i in range(4)]

    lane = jax.lax.broadcasted_iota(i32, (8, 128), 1)

    def layer_norms(j, dep=None):
        n16 = D // 16
        k0 = jnp.broadcast_to(_unpack(x_s[0:8, lt(j)], 0)[0:1, :], (8, 128))
        if dep is not None:
            k0 = k0 + _zero_after(dep)
        s1, s2 = [None, None], [None, None]
        for i in range(n16):
            p = x_s[8 * i:8 * i + 8, lt(j)]
            for t in range(2):
                c = _unpack(p, t) - k0
                s1[t] = c if s1[t] is None else s1[t] + c
                s2[t] = c * c if s2[t] is None else s2[t] + c * c
        m1 = _col_sum(s1[0] + s1[1]) * (1.0 / D)
        m2 = _col_sum(s2[0] + s2[1]) * (1.0 / D)
        mean = k0 + m1
        rstd = jax.lax.rsqrt(jnp.maximum(m2 - m1 * m1, 0.0) + EPS)
        t1, t2 = [None, None], [None, None]
        for i in range(n16):
            p = x_s[8 * i:8 * i + 8, lt(j)]
            xs = []
            for t in range(2):
                xn = (_unpack_bits(p, t) - mean) * rstd
                xs.append(xn)
                t1[t] = xn if t1[t] is None else t1[t] + xn
                t2[t] = xn * xn if t2[t] is None else t2[t] + xn * xn
            xn_s[8 * i:8 * i + 8, lt(j)] = _pack(xs[0], xs[1])
        mean2 = _col_sum(t1[0] + t1[1]) * (1.0 / D)
        e2 = _col_sum(t2[0] + t2[1]) * (1.0 / D)
        rstd2 = jax.lax.rsqrt(jnp.maximum(e2 - mean2 * mean2, 0.0) + EPS)
        for i in range(n16):
            p = xn_s[8 * i:8 * i + 8, lt(j)]
            h_s[8 * i:8 * i + 8, lt(j)] = _pack((_unpack(p, 0) - mean2) * rstd2, (_unpack(p, 1) - mean2) * rstd2)
        return rstd2

    def prep_wqkv(c, dep):
        rows = min(128, D - 128 * c)
        wp = wqkv_s[64 * c:64 * c + rows // 2, :]
        wp = jnp.where(jnp.tile(_never(dep), (rows // 16, 11))[:, :3 * D], jnp.uint32(0), wp)
        w = _as_bf16(wp).astype(f32)
        if rows < 128:
            w = jnp.concatenate([w, jnp.zeros((128 - rows, 3 * D), f32)], axis=0)
        wt = w.T
        for v in range(3 * D // 8):
            wt_f[c, pl.ds(8 * v + (8 * v) // (2 * DH), 8), :] = wt[8 * v:8 * v + 8]
        for sec in range(3):
            for d in range(DH):
                even, odd = (wt_f[c, pl.ds(sec * 8 * ST + DH * g + d, 8, stride=ST), :] for g in range(2))
                wt_s[c, sec * (D // 2) + 8 * d:sec * (D // 2) + 8 * d + 8, :] = _pack(even, odd)

    def prep_wo(c, dep):
        cols = min(128, D - 128 * c)
        wp = wo_s[:, 128 * c:128 * c + cols]
        wp = jnp.where(jnp.tile(_never(dep), (D // 16, 1))[:, :cols], jnp.uint32(0), wp)
        if cols < 128:
            wp = jnp.concatenate([wp, jnp.zeros((D // 2, 128 - cols), u32)], axis=1)
        wo_f[c, 0:D // 2, :] = wp
        parts = []
        for e in range(DH // 2):
            g0, g1 = (wo_f[c, pl.ds(14 * 8 * g + e, 8, stride=14), :] for g in range(2))
            for t in range(2):
                parts.append(_pack(_unpack(g0, t), _unpack(g1, t)))
        wpk = _as_bf16(jnp.concatenate(parts, axis=0))
        wpk = jnp.concatenate([wpk, jnp.zeros((512 - D, 128), bf16)], axis=0)
        wpt = pltpu.bitcast(wpk.T, u32)
        rows = min(128, D - 128 * c) // 2
        for cc in range(4):
            wot_s[cc, 64 * c:64 * c + rows, :] = wpt[:rows, lt(cc)]

    def lhs_448(ref):
        return jnp.concatenate([_as_bf16(ref[0]), _as_bf16(ref[1]), _as_bf16(ref[2]),
                                _as_bf16(ref[3])[:, 0:64]], axis=1)

    def qkv(j):
        res = jnp.dot(lhs_448(wt_s), _as_bf16(xn_s[:, lt(j)]), preferred_element_type=f32)
        q_s[j] = res[0:D]
        for dst, r0 in ((k_s, D), (v_s, 2 * D)):
            for d in range(DH):
                dst[j, 8 * d:8 * d + 8, :] = _pack(res[r0 + 16 * d:r0 + 16 * d + 8], res[r0 + 16 * d + 8:r0 + 16 * d + 16])
        return [res[s * D:s * D + 8] for s in range(3)]

    def shifted(cur, prev, w):
        sh = DIL * w
        return pltpu.roll(jnp.where(lane >= 128 - sh, prev, cur), sh, 1)

    def attention(j):
        jp = max(j - 1, 0)
        acc = [[None, None] for _ in range(W)]
        hist = []
        for d in range(DH):
            q = [q_s[j, 16 * d + 8 * g:16 * d + 8 * g + 8, :] for g in range(2)]
            k = k_s[j, 8 * d:8 * d + 8, :]
            kp = k_s[jp, 8 * d:8 * d + 8, :]
            krot = k
            if d >= 2:
                krot = jnp.where(_never(hist[d - 2]), jnp.uint32(0), k)
            for w in range(W):
                ks = k if w == 0 else shifted(krot, kp, w)
                for g in range(2):
                    p = q[g] * _unpack(ks, g)
                    acc[w][g] = p if acc[w][g] is None else acc[w][g] + p
            hist.append(acc[0][1])
        scale = DH ** -0.5
        prob = [[None, None] for _ in range(W)]
        for g in range(2):
            lg = [acc[w][g] for w in range(W)]
            if j == 0:
                lg = [lg[w] if w == 0 else jnp.where(lane >= DIL * w, lg[w], -1e9 / scale) for w in range(W)]
            m = lg[0]
            for w in range(1, W):
                m = jnp.maximum(m, lg[w])
            e = [jnp.exp2((t - m) * (scale * 1.4426950408889634)) for t in lg]
            esum = _tree_sum(e)
            inv = 1.0 / esum
            for w in range(W):
                prob[w][g] = e[w] * inv
        hold = _never(esum)
        for d in range(DH):
            v = jnp.where(hold, jnp.uint32(0), v_s[j, 8 * d:8 * d + 8, :])
            vp = v_s[jp, 8 * d:8 * d + 8, :]
            o = [None, None]
            for w in range(W):
                vs = v if w == 0 else shifted(v, vp, w)
                for g in range(2):
                    p = prob[w][g] * _unpack(vs, g)
                    o[g] = p if o[g] is None else o[g] + p
            o_s[j, 8 * d:8 * d + 8, :] = _pack(o[0], o[1])

    def oproj(j):
        a = jnp.dot(lhs_448(wot_s), _as_bf16(o_s[j]), preferred_element_type=f32)
        b2 = b2_s[pl.ds(128 * j, 128)].astype(f32).reshape(1, 128)
        r_s[j] = a + _as_bf16(x_s[:, lt(j)]).astype(f32) + b2

    def mixer_up(t0, nt, c0, nc):
        hb = _as_bf16(h_s[:, lt(t0, nt)])
        wb = _as_bf16(w1_s[64 * t0:64 * (t0 + nt), lt(c0, nc)])
        upd = jnp.dot(hb, wb, preferred_element_type=f32)
        if t0 == 0:
            u_s[:, lt(c0, nc)] = upd
        elif t0 + nt < NT:
            u_s[:, lt(c0, nc)] = u_s[:, lt(c0, nc)] + upd
        else:
            b1 = b1_s[pl.ds(128 * c0, 128 * nc)].astype(f32).reshape(1, 128 * nc)
            t = u_s[:, lt(c0, nc)] + upd + b1
            ub_s[:, lt(c0, nc)] = pltpu.bitcast(jax.nn.gelu(t, approximate=True).astype(bf16), u32)
        return upd[0:8, 0:128]

    def mixer_down(j0):
        if isinstance(j0, int):
            cols = lambda t, n: lt(j0 + t, n)
        else:
            cols = lambda t, n: pl.ds(pl.multiple_of((j0 + t) * 128, 128), 128 * n)
        y = jnp.dot(_as_bf16(ub_s[...]), _as_bf16(w2_s[:, cols(0, 2)]), preferred_element_type=f32)
        for t in range(2):
            out_s[:, cols(t, 1)] = pltpu.bitcast((y[:, lt(t)] + r_s[j0 + t]).astype(bf16), u32)

    def out_copy(j0, n, sem):
        sl = lt(j0, n) if isinstance(j0, int) else pl.ds(pl.multiple_of(j0 * 128, 128), 128 * n)
        return pltpu.make_async_copy(out_s.at[:, sl], out_hbm.at[:, sl], sems.at[sem])

    cp_x[0].wait()
    tok = layer_norms(0)
    for p, piece in enumerate(START):
        for c in cp_start.get(p, ()):
            c.wait(tok)
        tok = [mixer_up(*dot) for dot in piece][0]
        for j, at in LN_IN_START.items():
            if at == p:
                if j in cp_x:
                    cp_x[j].wait(tok)
                layer_norms(j, tok)
        for i in range(4):
            if WQKV_PREP_AT[i] == p:
                cp_wqkv[i].wait(tok)
                prep_wqkv(i, tok)

    for b in range(NB):
        for t, j in enumerate(range(KB * b, KB * b + KB)):
            toks = qkv(j)
            if b == 0:
                for jj, at in LN_IN_QKV.items():
                    if at // 3 == t:
                        layer_norms(jj, toks[at % 3])
            if t == KB - 1:
                cp_w1[b].wait(toks[1])
                if b == 0:
                    cp_x[12].wait(toks[1])
                if b == 2:
                    cp_b1.wait(toks[1])
                if b == NB - 1:
                    for c in cp_w2:
                        c.wait(toks[1])
            attention(j)
        for i in range(7):
            tok = mixer_up(KB * (2 + b // 2), KB, 7 * (b % 2) + i, 1)
            if b == 1:
                for jj, at in LN_IN_FILL.items():
                    if at == i:
                        layer_norms(jj, tok)
            if b == 0:
                for c in range(4):
                    if WO_PREP_AT[c] == i:
                        if c == 0:
                            cp_wo.wait(tok)
                            cp_b2.wait(tok)
                        prep_wo(c, tok)
        for j in range(KB * b, KB * b + KB):
            oproj(j)

    s0 = n_sem[0]
    mixer_down(0)
    out_copy(0, 2, s0).start()

    def body(i, carry):
        j0 = 2 + 2 * LOOP_P * i
        for p in range(LOOP_P):
            mixer_down(j0 + 2 * p)
        out_copy(j0, 2 * LOOP_P, s0 + 1 + i).start()
        return carry

    jax.lax.fori_loop(0, LOOP_N, body, 0)
    jt = 2 + 2 * LOOP_P * LOOP_N
    mixer_down(jt)
    out_copy(jt, NT - jt, s0 + 1 + LOOP_N).start()
    out_copy(0, 2, s0).wait()
    for i in range(LOOP_N):
        out_copy(2 + 2 * LOOP_P * i, 2 * LOOP_P, s0 + 1 + i).wait()
    out_copy(jt, NT - jt, s0 + 1 + LOOP_N).wait()


@jax.jit
def pallas_parallel_sum__sliding_local_dilated__mixer_token_mlp__prompt_kernel(
    A_x, A_wqkv, A_wo, B_x, B_w1, B_b1, B_w2, B_b2,
):
    del B_x
    xT = A_x.reshape(S, D).T
    any_spec = pl.BlockSpec(memory_space=pl.ANY)
    scratch = [
        pltpu.VMEM((D // 2, S), u32),
        pltpu.VMEM((D // 2, 3 * D), u32),
        pltpu.VMEM((D // 2, D), u32),
        pltpu.VMEM((S // 2, F), u32),
        pltpu.VMEM((F // 2, S), u32),
        pltpu.VMEM((F,), bf16),
        pltpu.VMEM((S,), bf16),
        pltpu.VMEM((4, 25 * ST + 7, 128), f32),
        pltpu.VMEM((4, D // 2 + 16, 128), u32),
        pltpu.VMEM((4, 3 * D // 2, 128), u32),
        pltpu.VMEM((4, D // 2, 128), u32),
        pltpu.VMEM((D // 2, S), u32),
        pltpu.VMEM((D // 2, S), u32),
        pltpu.VMEM((NT, D, 128), f32),
        pltpu.VMEM((NT, D // 2, 128), u32),
        pltpu.VMEM((NT, D // 2, 128), u32),
        pltpu.VMEM((NT, D // 2, 128), u32),
        pltpu.VMEM((NT, D, 128), f32),
        pltpu.VMEM((D, F), f32),
        pltpu.VMEM((D // 2, F), u32),
        pltpu.VMEM((D // 2, S), u32),
        pltpu.SemaphoreType.DMA((N_SEMS,)),
    ]
    outT = pl.pallas_call(
        _kernel,
        out_shape=jax.ShapeDtypeStruct((D, S), bf16),
        in_specs=[any_spec] * 7,
        out_specs=any_spec,
        scratch_shapes=scratch,
        compiler_params=pltpu.CompilerParams(
            vmem_limit_bytes=64 * 1024 * 1024,
            flags={"XLA_TPU_RESCHEDULE_DMA_DONES": True, "XLA_TPU_EVENLY_DISTRIBUTE_CRITICAL_NODES": True},
            disable_semaphore_checks=True,
        ),
        name="fused_kernel",
    )(xT, A_wqkv, A_wo, B_w1, B_b1, B_w2, B_b2)
    return outT.T.reshape(1, S, D)
```

```python
import jax
import jax.numpy as jnp
import jax.experimental.pallas as pl
import jax.experimental.pallas.tpu as pltpu

S, D, H, DH, F = 2048, 448, 16, 28, 1792
W, DIL = 8, 2
NT = S // 128
NF = F // 128
KB = 4
NB = NT // KB
EPS = 1e-5
ST = 57
f32, bf16, u32, i32 = jnp.float32, jnp.bfloat16, jnp.uint32, jnp.int32

START = ([[(0, 1, 0, 4)], [(0, 1, 4, 4)], [(0, 1, 8, 4)], [(0, 1, 12, 2), (1, 1, 0, 2)],
          [(1, 1, 2, 4)], [(1, 1, 6, 4)], [(1, 1, 10, 4)]]
         + [[(2, 2, 2 * i, 2)] for i in range(NF // 2)]
         + [[(4, 4, c, 1)] for c in range(NF)])
LN_IN_START = {1: 1, 2: 4, 3: 5, 4: 8, 5: 10, 6: 11, 7: 12, 8: 27}
LN_IN_QKV = {9: 0, 10: 1, 11: 2}
LN_IN_FILL = {12: 3, 13: 4, 14: 5, 15: 6}
WQKV_PREP_AT = (14, 18, 21, 25)
WO_PREP_AT = (2, 3, 4, 5)
TAIL_ROWS = 192
LOOP_N, LOOP_P = 2, 3
N_SEMS = 49


def _unpack(x, i):
    return pltpu.unpack_elementwise(x, index=i, packed_dtype=bf16, unpacked_dtype=f32)


def _unpack_bits(x, i):
    if i == 0:
        return jax.lax.bitcast_convert_type(x << 16, f32)
    return jax.lax.bitcast_convert_type(x & jnp.uint32(0xFFFF0000), f32)


def _pack(lo, hi):
    return pltpu.pack_elementwise([lo, hi], packed_dtype=bf16)


def _as_bf16(x_u32):
    return pltpu.bitcast(x_u32, bf16)


def _tree_sum(xs):
    xs = list(xs)
    while len(xs) > 1:
        nxt = [xs[i] + xs[i + 1] for i in range(0, len(xs) - 1, 2)]
        if len(xs) % 2:
            nxt.append(xs[-1])
        xs = nxt
    return xs[0]


def _col_sum(p):
    return jnp.broadcast_to(jnp.sum(p, axis=0, keepdims=True), (8, 128))


def _never(tok):
    return tok * tok < -1.0


def _zero_after(tok):
    return jnp.where(_never(tok), 1.0, 0.0).astype(f32)


def _kernel(x_hbm, wqkv_hbm, wo_hbm, w1_hbm, b1_hbm, w2_hbm, b2_hbm, out_hbm,
            x_s, wqkv_s, wo_s, w1_s, w2_s, b1_s, b2_s,
            wt_f, wo_f, wt_s, wot_s,
            xn_s, h_s, q_s, k_s, v_s, o_s, r_s, u_s, ub_s, out_s, sems):
    x_hbm, wqkv_hbm, wo_hbm, w1_hbm, w2_hbm, out_hbm = (
        r.bitcast(u32) for r in (x_hbm, wqkv_hbm, wo_hbm, w1_hbm, w2_hbm, out_hbm))

    def lt(j, n=1):
        return slice(128 * j, 128 * (j + n))

    n_sem = [0]

    class Dma:
        def __init__(self, src, dst):
            self.src, self.dst, self.sem = src, dst, n_sem[0]
            n_sem[0] += 1
            pltpu.make_async_copy(src, dst, sems.at[self.sem]).start()

        def wait(self, tok=None):
            sem = self.sem
            if tok is not None:
                sem = sem + jnp.where(_never(tok), 1, 0).astype(i32)[0, 0]
            pltpu.make_async_copy(self.src, self.dst, sems.at[sem]).wait()

    def x_dma(j, n):
        return Dma(x_hbm.at[:, lt(j, n)], x_s.at[:, lt(j, n)])

    def w1_dma(t0, nt, c0, nc):
        rows = pl.ds(64 * t0, 64 * nt)
        return Dma(w1_hbm.at[rows, lt(c0, nc)], w1_s.at[rows, lt(c0, nc)])

    def wqkv_dma(c):
        rows = pl.ds(64 * c, min(64, D // 2 - 64 * c))
        return Dma(wqkv_hbm.at[rows], wqkv_s.at[rows])

    cp_x = {0: x_dma(0, 1)}
    cp_start = {}
    for p in range(7):
        cp_start[p] = [w1_dma(*dot) for dot in START[p]]
        if p in (1, 5, 6):
            j = {1: 1, 5: 2, 6: 3}[p]
            cp_x[j] = x_dma(j, 1)
    for i in range(7):
        cp_start[7 + i] = [w1_dma(2, 2, 2 * i, 2)]
        if i == 1:
            cp_x[4] = x_dma(4, 4)
    cp_wqkv = []
    for i in range(7):
        cp_start[14 + 2 * i] = [w1_dma(4, 4, 2 * i, 2)]
        if i in (0, 2, 3, 5):
            cp_wqkv.append(wqkv_dma(len(cp_wqkv)))
    cp_x[8] = x_dma(8, 4)
    cp_wo = Dma(wo_hbm, wo_s)
    cp_b2 = Dma(b2_hbm, b2_s)
    cp_x[12] = x_dma(12, 4)
    cp_b1 = Dma(b1_hbm, b1_s)
    cp_w1 = [w1_dma(KB * (2 + b // 2), KB, 7 * (b % 2), 7) for b in range(NB)]
    cp_w2 = [Dma(w2_hbm.at[:, lt(4 * i, 4)], w2_s.at[:, lt(4 * i, 4)]) for i in range(4)]

    lane = jax.lax.broadcasted_iota(i32, (8, 128), 1)

    def layer_norms(j, dep=None):
        n16 = D // 16
        k0 = jnp.broadcast_to(_unpack(x_s[0:8, lt(j)], 0)[0:1, :], (8, 128))
        if dep is not None:
            k0 = k0 + _zero_after(dep)
        s1, s2 = [None, None], [None, None]
        for i in range(n16):
            p = x_s[8 * i:8 * i + 8, lt(j)]
            for t in range(2):
                c = _unpack(p, t) - k0
                s1[t] = c if s1[t] is None else s1[t] + c
                s2[t] = c * c if s2[t] is None else s2[t] + c * c
        m1 = _col_sum(s1[0] + s1[1]) * (1.0 / D)
        m2 = _col_sum(s2[0] + s2[1]) * (1.0 / D)
        mean = k0 + m1
        rstd = jax.lax.rsqrt(jnp.maximum(m2 - m1 * m1, 0.0) + EPS)
        t1, t2 = [None, None], [None, None]
        for i in range(n16):
            p = x_s[8 * i:8 * i + 8, lt(j)]
            xs = []
            for t in range(2):
                xn = (_unpack_bits(p, t) - mean) * rstd
                xs.append(xn)
                t1[t] = xn if t1[t] is None else t1[t] + xn
                t2[t] = xn * xn if t2[t] is None else t2[t] + xn * xn
            xn_s[8 * i:8 * i + 8, lt(j)] = _pack(xs[0], xs[1])
        mean2 = _col_sum(t1[0] + t1[1]) * (1.0 / D)
        e2 = _col_sum(t2[0] + t2[1]) * (1.0 / D)
        rstd2 = jax.lax.rsqrt(jnp.maximum(e2 - mean2 * mean2, 0.0) + EPS)
        for i in range(n16):
            p = xn_s[8 * i:8 * i + 8, lt(j)]
            h_s[8 * i:8 * i + 8, lt(j)] = _pack((_unpack(p, 0) - mean2) * rstd2, (_unpack(p, 1) - mean2) * rstd2)
        return rstd2

    def prep_wqkv(c, dep):
        rows = min(128, D - 128 * c)
        wp = wqkv_s[64 * c:64 * c + rows // 2, :]
        wp = jnp.where(jnp.tile(_never(dep), (rows // 16, 11))[:, :3 * D], jnp.uint32(0), wp)
        w = _as_bf16(wp).astype(f32)
        if rows < 128:
            w = jnp.concatenate([w, jnp.zeros((128 - rows, 3 * D), f32)], axis=0)
        wt = w.T
        for v in range(3 * D // 8):
            wt_f[c, pl.ds(8 * v + (8 * v) // (2 * DH), 8), :] = wt[8 * v:8 * v + 8]
        for sec in range(3):
            for d in range(DH):
                even, odd = (wt_f[c, pl.ds(sec * 8 * ST + DH * g + d, 8, stride=ST), :] for g in range(2))
                wt_s[c, sec * (D // 2) + 8 * d:sec * (D // 2) + 8 * d + 8, :] = _pack(even, odd)

    def prep_wo(c, dep):
        cols = min(128, D - 128 * c)
        wp = wo_s[:, 128 * c:128 * c + cols]
        wp = jnp.where(jnp.tile(_never(dep), (D // 16, 1))[:, :cols], jnp.uint32(0), wp)
        if cols < 128:
            wp = jnp.concatenate([wp, jnp.zeros((D // 2, 128 - cols), u32)], axis=1)
        wo_f[c, 0:D // 2, :] = wp
        parts = []
        for e in range(DH // 2):
            g0, g1 = (wo_f[c, pl.ds(14 * 8 * g + e, 8, stride=14), :] for g in range(2))
            for t in range(2):
                parts.append(_pack(_unpack(g0, t), _unpack(g1, t)))
        wpk = _as_bf16(jnp.concatenate(parts, axis=0))
        wpk = jnp.concatenate([wpk, jnp.zeros((512 - D, 128), bf16)], axis=0)
        wpt = pltpu.bitcast(wpk.T, u32)
        rows = min(128, D - 128 * c) // 2
        for cc in range(4):
            wot_s[cc, 64 * c:64 * c + rows, :] = wpt[:rows, lt(cc)]

    def lhs_448(ref):
        return jnp.concatenate([_as_bf16(ref[0]), _as_bf16(ref[1]), _as_bf16(ref[2]),
                                _as_bf16(ref[3])[:, 0:64]], axis=1)

    def qkv(j):
        res = jnp.dot(lhs_448(wt_s), _as_bf16(xn_s[:, lt(j)]), preferred_element_type=f32)
        q_s[j] = res[0:D]
        for dst, r0 in ((k_s, D), (v_s, 2 * D)):
            for d in range(DH):
                dst[j, 8 * d:8 * d + 8, :] = _pack(res[r0 + 16 * d:r0 + 16 * d + 8], res[r0 + 16 * d + 8:r0 + 16 * d + 16])
        return [res[s * D:s * D + 8] for s in range(3)]

    def shifted(cur, prev, w):
        sh = DIL * w
        return pltpu.roll(jnp.where(lane >= 128 - sh, prev, cur), sh, 1)

    def attention(j):
        jp = max(j - 1, 0)
        acc = [[None, None] for _ in range(W)]
        hist = []
        for d in range(DH):
            q = [q_s[j, 16 * d + 8 * g:16 * d + 8 * g + 8, :] for g in range(2)]
            k = k_s[j, 8 * d:8 * d + 8, :]
            kp = k_s[jp, 8 * d:8 * d + 8, :]
            krot = k
            if d >= 2:
                krot = jnp.where(_never(hist[d - 2]), jnp.uint32(0), k)
            for w in range(W):
                ks = k if w == 0 else shifted(krot, kp, w)
                for g in range(2):
                    p = q[g] * _unpack(ks, g)
                    acc[w][g] = p if acc[w][g] is None else acc[w][g] + p
            hist.append(acc[0][1])
        scale = DH ** -0.5
        prob = [[None, None] for _ in range(W)]
        for g in range(2):
            lg = [acc[w][g] for w in range(W)]
            if j == 0:
                lg = [lg[w] if w == 0 else jnp.where(lane >= DIL * w, lg[w], -1e9 / scale) for w in range(W)]
            m = lg[0]
            for w in range(1, W):
                m = jnp.maximum(m, lg[w])
            e = [jnp.exp2((t - m) * (scale * 1.4426950408889634)) for t in lg]
            esum = _tree_sum(e)
            inv = 1.0 / esum
            for w in range(W):
                prob[w][g] = e[w] * inv
        hold = _never(esum)
        for d in range(DH):
            v = jnp.where(hold, jnp.uint32(0), v_s[j, 8 * d:8 * d + 8, :])
            vp = v_s[jp, 8 * d:8 * d + 8, :]
            o = [None, None]
            for w in range(W):
                vs = v if w == 0 else shifted(v, vp, w)
                for g in range(2):
                    p = prob[w][g] * _unpack(vs, g)
                    o[g] = p if o[g] is None else o[g] + p
            o_s[j, 8 * d:8 * d + 8, :] = _pack(o[0], o[1])

    def oproj(j):
        a = jnp.dot(lhs_448(wot_s), _as_bf16(o_s[j]), preferred_element_type=f32)
        b2 = b2_s[pl.ds(128 * j, 128)].astype(f32).reshape(1, 128)
        r_s[j] = a + _as_bf16(x_s[:, lt(j)]).astype(f32) + b2

    def mixer_up(t0, nt, c0, nc):
        hb = _as_bf16(h_s[:, lt(t0, nt)])
        wb = _as_bf16(w1_s[64 * t0:64 * (t0 + nt), lt(c0, nc)])
        upd = jnp.dot(hb, wb, preferred_element_type=f32)
        if t0 == 0:
            u_s[:, lt(c0, nc)] = upd
        elif t0 + nt < NT:
            u_s[:, lt(c0, nc)] = u_s[:, lt(c0, nc)] + upd
        else:
            b1 = b1_s[pl.ds(128 * c0, 128 * nc)].astype(f32).reshape(1, 128 * nc)
            t = u_s[:, lt(c0, nc)] + upd + b1
            ub_s[:, lt(c0, nc)] = pltpu.bitcast(jax.nn.gelu(t, approximate=True).astype(bf16), u32)
        return upd[0:8, 0:128]

    def mixer_down(j0, r0=0, nr=D):
        if isinstance(j0, int):
            cols = lambda t, n: lt(j0 + t, n)
        else:
            cols = lambda t, n: pl.ds(pl.multiple_of((j0 + t) * 128, 128), 128 * n)
        rw = slice(r0 // 2, (r0 + nr) // 2)
        y = jnp.dot(_as_bf16(ub_s[rw, :]), _as_bf16(w2_s[:, cols(0, 2)]), preferred_element_type=f32)
        for t in range(2):
            out_s[rw, cols(t, 1)] = pltpu.bitcast((y[:, lt(t)] + r_s[j0 + t, r0:r0 + nr, :]).astype(bf16), u32)

    def out_copy(j0, n, sem, r0=0, nr=D):
        sl = lt(j0, n) if isinstance(j0, int) else pl.ds(pl.multiple_of(j0 * 128, 128), 128 * n)
        rw = slice(r0 // 2, (r0 + nr) // 2)
        return pltpu.make_async_copy(out_s.at[rw, sl], out_hbm.at[rw, sl], sems.at[sem])

    cp_x[0].wait()
    tok = layer_norms(0)
    for p, piece in enumerate(START):
        for c in cp_start.get(p, ()):
            c.wait(tok)
        tok = [mixer_up(*dot) for dot in piece][0]
        for j, at in LN_IN_START.items():
            if at == p:
                if j in cp_x:
                    cp_x[j].wait(tok)
                layer_norms(j, tok)
        for i in range(4):
            if WQKV_PREP_AT[i] == p:
                cp_wqkv[i].wait(tok)
                prep_wqkv(i, tok)

    for b in range(NB):
        for t, j in enumerate(range(KB * b, KB * b + KB)):
            toks = qkv(j)
            if b == 0:
                for jj, at in LN_IN_QKV.items():
                    if at // 3 == t:
                        layer_norms(jj, toks[at % 3])
            if t == KB - 1:
                cp_w1[b].wait(toks[1])
                if b == 0:
                    cp_x[12].wait(toks[1])
                if b == 2:
                    cp_b1.wait(toks[1])
                if b == NB - 1:
                    for c in cp_w2:
                        c.wait(toks[1])
            attention(j)
        for i in range(7):
            tok = mixer_up(KB * (2 + b // 2), KB, 7 * (b % 2) + i, 1)
            if b == 1:
                for jj, at in LN_IN_FILL.items():
                    if at == i:
                        layer_norms(jj, tok)
            if b == 0:
                for c in range(4):
                    if WO_PREP_AT[c] == i:
                        if c == 0:
                            cp_wo.wait(tok)
                            cp_b2.wait(tok)
                        prep_wo(c, tok)
        for j in range(KB * b, KB * b + KB):
            oproj(j)

    s0 = n_sem[0]
    jt, rh = NT - 2, D - TAIL_ROWS
    mixer_down(0)
    mixer_down(jt, 0, rh)
    out_copy(0, 2, s0).start()
    out_copy(jt, 2, s0 + 1, 0, rh).start()

    def body(i, carry):
        j0 = 2 + 2 * LOOP_P * i
        for p in range(LOOP_P):
            mixer_down(j0 + 2 * p)
        out_copy(j0, 2 * LOOP_P, s0 + 2 + i).start()
        return carry

    jax.lax.fori_loop(0, LOOP_N, body, 0)
    mixer_down(jt, rh, TAIL_ROWS)
    out_copy(jt, 2, s0 + 2 + LOOP_N, rh, TAIL_ROWS).start()
    out_copy(0, 2, s0).wait()
    out_copy(jt, 2, s0 + 1, 0, rh).wait()
    for i in range(LOOP_N):
        out_copy(2 + 2 * LOOP_P * i, 2 * LOOP_P, s0 + 2 + i).wait()
    out_copy(jt, 2, s0 + 2 + LOOP_N, rh, TAIL_ROWS).wait()


@jax.jit
def pallas_parallel_sum__sliding_local_dilated__mixer_token_mlp__prompt_kernel(
    A_x, A_wqkv, A_wo, B_x, B_w1, B_b1, B_w2, B_b2,
):
    del B_x
    xT = A_x.reshape(S, D).T
    any_spec = pl.BlockSpec(memory_space=pl.ANY)
    scratch = [
        pltpu.VMEM((D // 2, S), u32),
        pltpu.VMEM((D // 2, 3 * D), u32),
        pltpu.VMEM((D // 2, D), u32),
        pltpu.VMEM((S // 2, F), u32),
        pltpu.VMEM((F // 2, S), u32),
        pltpu.VMEM((F,), bf16),
        pltpu.VMEM((S,), bf16),
        pltpu.VMEM((4, 25 * ST + 7, 128), f32),
        pltpu.VMEM((4, D // 2 + 16, 128), u32),
        pltpu.VMEM((4, 3 * D // 2, 128), u32),
        pltpu.VMEM((4, D // 2, 128), u32),
        pltpu.VMEM((D // 2, S), u32),
        pltpu.VMEM((D // 2, S), u32),
        pltpu.VMEM((NT, D, 128), f32),
        pltpu.VMEM((NT, D // 2, 128), u32),
        pltpu.VMEM((NT, D // 2, 128), u32),
        pltpu.VMEM((NT, D // 2, 128), u32),
        pltpu.VMEM((NT, D, 128), f32),
        pltpu.VMEM((D, F), f32),
        pltpu.VMEM((D // 2, F), u32),
        pltpu.VMEM((D // 2, S), u32),
        pltpu.SemaphoreType.DMA((N_SEMS,)),
    ]
    outT = pl.pallas_call(
        _kernel,
        out_shape=jax.ShapeDtypeStruct((D, S), bf16),
        in_specs=[any_spec] * 7,
        out_specs=any_spec,
        scratch_shapes=scratch,
        compiler_params=pltpu.CompilerParams(
            vmem_limit_bytes=64 * 1024 * 1024,
            flags={"XLA_TPU_RESCHEDULE_DMA_DONES": True, "XLA_TPU_EVENLY_DISTRIBUTE_CRITICAL_NODES": True},
            disable_semaphore_checks=True,
        ),
        name="fused_kernel",
    )(xT, A_wqkv, A_wo, B_w1, B_b1, B_w2, B_b2)
    return outT.T.reshape(1, S, D)
```
